```python
import os as _os
_os.environ.setdefault('JAX_PLATFORMS', 'cpu')
import jax
import jax.numpy as jnp

def _softmax(x, axis=-1):
    return jax.nn.softmax(x, axis=axis)

def _gelu(x):
    return jax.nn.gelu(x, approximate=True)

def _silu(x):
    return jax.nn.silu(x)

def _sigmoid(x):
    return jax.nn.sigmoid(x)

def _layernorm(x, axis=-1, eps=1e-05):
    m = jnp.mean(x, axis=axis, keepdims=True)
    v = jnp.var(x, axis=axis, keepdims=True)
    return (x - m) / jnp.sqrt(v + eps)

def _scatter_add(tgt, idx, src, axis=0):
    return tgt.at[idx].add(src)

def _segment_sum(src, seg, n):
    return jax.ops.segment_sum(src, seg, n)

class _Rng:

    def __init__(self, key):
        self._k = key

    def _next(self):
        self._k, sub = jax.random.split(self._k)
        return sub

    def normal(self, shape):
        return jax.random.normal(self._next(), shape, dtype=jnp.bfloat16)

    def randint(self, lo, hi, shape):
        return jax.random.randint(self._next(), shape, lo, hi, dtype=jnp.int32)

    def uniform(self, shape, lo=0.0, hi=1.0):
        return jax.random.uniform(self._next(), shape, jnp.bfloat16, lo, hi)

    def permutation(self, n):
        return jax.random.permutation(self._next(), n)
kernel_name = 'adaLN_cond__sliding_block__mixer_channel_mlp__prompt'

def setup_inputs():
    _rng = _Rng(jax.random.key(int.from_bytes(__import__("os").urandom(4), "little")))
    _w = lambda a: (lambda t: t.astype(jnp.bfloat16) if jnp.issubdtype(t.dtype, jnp.floating) else t)(jnp.asarray(a))

    def _A_setup():
        B, S, D = (1, 2048, 640)
        return {'x': _w((lambda *s: _rng.normal(s) * 0.05)(B, S, D)), 'wqkv': _w((lambda *s: _rng.normal(s) * 0.05)(D, 3 * D)), 'wo': _w((lambda *s: _rng.normal(s) * 0.05)(D, D))}
    _A_in = _A_setup()

    def _B_setup():
        B, S, D, F = (1, 2048, 640, 1728)
        return {'x': _w((lambda *s: _rng.normal(s) * 0.05)(B, S, D)), 'w1': _w((lambda *s: _rng.normal(s) * 0.8)(D, F) * D ** (-0.5)), 'b1': _w((lambda *s: _rng.normal(s) * 0.8)(F)), 'w2': _w((lambda *s: _rng.normal(s) * 0.8)(F, D) * F ** (-0.5)), 'b2': _w((lambda *s: _rng.normal(s) * 0.4)(D))}
    _B_in = _B_setup()
    return {'A_x': _A_in['x'], 'A_wqkv': _A_in['wqkv'], 'A_wo': _A_in['wo'], 'B_x': _B_in['x'], 'B_w1': _B_in['w1'], 'B_b1': _B_in['b1'], 'B_w2': _B_in['w2'], 'B_b2': _B_in['b2'], 'c': _w((lambda *s: _rng.normal(s) * 0.05)(1, 640) * 8.0), 'w_mod': _w((lambda *s: _rng.normal(s) * 0.05)(640, 6 * 640) * 640 ** (-0.5) * 8.0)}

def reference(A_x, A_wqkv, A_wo, B_x, B_w1, B_b1, B_w2, B_b2, c, w_mod):

    def _A_ref(x, wqkv, wo):
        B, S, D = x.shape
        H = 32
        Dh = D // H
        W = 256
        qkv = (lambda x, *d: x.transpose(*d))((x @ wqkv).reshape(B, S, 3, H, Dh), 2, 0, 3, 1, 4)
        q, k, v = (qkv[0], qkv[1], qkv[2])
        scores = jnp.einsum('bhqd,bhkd->bhqk', q, k) * Dh ** (-0.5)
        idx = jnp.arange(S)
        mask = (idx[:, None] - idx[None, :] >= 0) & (idx[:, None] - idx[None, :] < W)
        scores = jnp.where(mask[None, None], scores, -1000000000.0)
        p = _softmax(scores, axis=-1)
        o = jnp.einsum('bhqk,bhkd->bhqd', p, v)
        return (lambda x, *d: x.transpose(*d))(o, 0, 2, 1, 3).reshape(B, S, D) @ wo

    def _B_ref(x, w1, b1, w2, b2):
        y = _layernorm(x, axis=-1)
        h = _gelu(jnp.einsum('bsd,df->bsf', y, w1) + b1)
        return jnp.einsum('bsf,fd->bsd', h, w2) + b2
    x = A_x
    mod = (_silu(c) @ w_mod).reshape(c.shape[0], 6, 1, -1)
    sa, ca, ga, sb, cb, gb = (mod[:, 0].copy(), mod[:, 1].copy(), mod[:, 2].copy(), mod[:, 3].copy(), mod[:, 4].copy(), mod[:, 5].copy())
    h = _layernorm(x, axis=-1) * (1 + ca) + sa
    x = x + ga * _A_ref(h, A_wqkv, A_wo)
    h = _layernorm(x, axis=-1) * (1 + cb) + sb
    x = x + gb * _B_ref(h, B_w1, B_b1, B_w2, B_b2)
    return x
```

```python
import functools
import math
import jax
import jax.numpy as jnp
from jax import lax
import jax.experimental.pallas as pl
import jax.experimental.pallas.tpu as pltpu

S = 2048
D = 640
H = 32
DH = 20
F = 1728
TM = 256
NB = S // TM
QB = 128
NQ = TM // QB
NG = 8
EPS = 1e-5
QSCALE = (DH ** -0.5) * math.log2(math.e)
NEG = -1e30
f32 = jnp.float32
bf16 = jnp.bfloat16
u32 = jnp.uint32
NT = (((1,), (1,)), ((), ()))


def _pk(a):
    return pltpu.bitcast(a.astype(bf16), u32)


def _upk(a):
    return pltpu.bitcast(a, bf16)


def _ln(x):
    mu = jnp.mean(x, axis=-1, keepdims=True)
    xc = x - mu
    var = jnp.mean(xc * xc, axis=-1, keepdims=True)
    return xc * lax.rsqrt(var + EPS)


def _group_tiles(a):
    m = a.shape[0]
    lane = lax.broadcasted_iota(jnp.int32, (m, 128), 1)
    hi = lane >= 64
    t = [a[:, 128 * j:128 * (j + 1)] for j in range(5)]
    out = []
    for g in range(NG):
        lo_t, hi_t = (80 * g) // 128, (80 * g + 79) // 128
        out.append(t[lo_t] if lo_t == hi_t else jnp.where(hi, t[lo_t], t[hi_t]))
    return out


def _kernel(x_hbm, wqkv_hbm, wo_hbm, w1T_hbm, b1_ref, w2_hbm, b2_ref, c_ref, wmod_hbm,
            o_ref,
            x_ref, wqkv_ref, wo_ref, w1T_ref, w2_ref, wmod_ref,
            mod_ref, bias_ref, wvT_ref, k_ref, q_ref, vT_ref, oT_ref, xsem, wsem):
    i = pl.program_id(0)

    def x_copy(b):
        return pltpu.make_async_copy(x_hbm.at[pl.ds(b * TM, TM)], x_ref.at[pl.ds(b * TM, TM)], xsem.at[b])

    def col_copy(src, dst, c0, n, s):
        return pltpu.make_async_copy(src.at[:, pl.ds(c0, n)], dst.at[:, pl.ds(c0, n)], wsem.at[s])

    cp_mod1 = col_copy(wmod_hbm, wmod_ref, 0, 2 * D, 0)
    cp_wq = col_copy(wqkv_hbm, wqkv_ref, 0, D, 1)
    cp_wk = col_copy(wqkv_hbm, wqkv_ref, D, D, 2)
    cp_wv = col_copy(wqkv_hbm, wqkv_ref, 2 * D, D, 3)
    cp_mod2 = col_copy(wmod_hbm, wmod_ref, 2 * D, 4 * D, 4)
    cp_wo = pltpu.make_async_copy(wo_hbm, wo_ref, wsem.at[5])
    cp_w1 = pltpu.make_async_copy(w1T_hbm, w1T_ref, wsem.at[6])
    cp_w2 = pltpu.make_async_copy(w2_hbm, w2_ref, wsem.at[7])

    def modrow(k):
        return mod_ref[0:1, k * D:(k + 1) * D]

    def silu_c():
        c = c_ref[...].astype(f32)
        sc = c * jax.nn.sigmoid(c)
        return jnp.broadcast_to(sc, (8, D)).astype(bf16)

    def load_x(b):
        return x_ref[pl.ds(pl.multiple_of(b * TM, TM), TM), :].astype(f32)

    def make_h(xn):
        return (xn * (1.0 + modrow(1)) + modrow(0)).astype(bf16)

    def proj_q(h):
        q = jnp.dot(h, wqkv_ref[:, 0:D], preferred_element_type=f32)
        qt = _group_tiles(_pk(q * QSCALE))
        for g in range(NG):
            q_ref[:, 128 * g:128 * (g + 1)] = qt[g]

    def proj_k(h, b):
        k = jnp.dot(h, wqkv_ref[:, D:2 * D], preferred_element_type=f32)
        row0 = pl.multiple_of(b * (TM // 2), TM // 2)
        kt = _group_tiles(_pk(k))
        for g in range(NG):
            k_ref[pl.ds(row0, TM // 2), 128 * g:128 * (g + 1)] = kt[g]

    def proj_v(h, b):
        vT = lax.dot_general(_upk(wvT_ref[...]), h, NT, preferred_element_type=f32)
        vTp = _pk(vT)
        r16 = lax.broadcasted_iota(jnp.int32, (16, QB), 0)
        ones = jnp.full((16, QB), 0x3F803F80, u32)
        for hd in range(H):
            base = (10 * hd) // 8 * 8
            off = 10 * hd - base
            useful = (r16 >= off) & (r16 < off + 10)
            for j in range(NQ):
                win = vTp[base:base + 16, QB * j:QB * (j + 1)]
                vT_ref[b * NQ + j, 16 * hd:16 * (hd + 1), :] = jnp.where(useful, win, ones)

    def attention(first):
        r64 = lax.broadcasted_iota(jnp.int32, (64, 128), 0)
        l64 = lax.broadcasted_iota(jnp.int32, (64, 128), 1)
        tri = r64 > (l64 & 63)
        left64 = l64 < 64
        kj = lax.broadcasted_iota(jnp.int32, (QB, QB), 0)
        qi = lax.broadcasted_iota(jnp.int32, (QB, QB), 1)
        uppers = (kj > qi, kj > (qi ^ 64))

        def nkeys(j):
            return min(j + 1, 3) if first else 3

        def stage_qk(j, g):
            jb = i * NQ + j
            nk = nkeys(j)
            cols = slice(128 * g, 128 * (g + 1))

            def krows(tile, a, n):
                st = pl.multiple_of((jb - 2 + tile) * 64 + a // 2, 8)
                return k_ref[pl.ds(st, n // 2), cols]

            qh = [_upk(q_ref[64 * j + 32 * half:64 * j + 32 * half + 32, cols]).astype(f32) for half in range(2)]

            def qmask(hd, half):
                st = (20 * hd) % 128
                return jnp.where(((l64 - st) & 127) < 20, qh[half], 0.0)

            def stat(lst):
                return jnp.concatenate([qmask(hd, half) for hd, half in lst], axis=0).astype(bf16)

            a, b, c_, d = range(4 * g, 4 * g + 4)
            q_lo = stat([(a, 0), (b, 0), (c_, 0), (d, 0)])
            q_hi = stat([(b, 1), (a, 1), (d, 1), (c_, 1)])
            p_lo, p_hi = [], []
            for c in range(4):
                if nk == 3:
                    p_lo += [krows(0, 16 * c, 16), krows(2, 16 * c, 16), krows(0, 64 + 16 * c, 16)]
                    p_hi += [krows(2, 16 * c, 16), krows(0, 64 + 16 * c, 16), krows(2, 64 + 16 * c, 16)]
                else:
                    p_lo += [krows(2, 16 * c, 16)]
                    p_hi += [krows(2, 16 * c, 16), krows(2, 64 + 16 * c, 16)]
            s_lo = lax.dot_general(_upk(jnp.concatenate(p_lo, axis=0)), q_lo, NT, preferred_element_type=f32)
            s_hi = lax.dot_general(_upk(jnp.concatenate(p_hi, axis=0)), q_hi, NT, preferred_element_type=f32)
            if nk >= 2:
                q_mid = stat([(a, 0), (a, 1), (b, 1), (b, 0), (c_, 0), (c_, 1), (d, 1), (d, 0)])
                s_mid = lax.dot_general(_upk(krows(1, 0, 128)), q_mid, NT, preferred_element_type=f32)

            def gather(s, k, n):
                return jnp.concatenate([s[16 * (n * c + k):16 * (n * c + k) + 16] for c in range(4)], axis=0)

            res = []
            for t in range(2):
                lo = s_lo[:, 128 * t:128 * (t + 1)]
                hi = s_hi[:, 128 * t:128 * (t + 1)]
                if nk == 3:
                    x_lo = jnp.where(tri, gather(lo, 0, 3), gather(lo, 1, 3))
                    f_lo = gather(lo, 2, 3)
                    f_hi = gather(hi, 0, 3)
                    x_hi = jnp.where(tri, gather(hi, 1, 3), gather(hi, 2, 3))
                else:
                    x_lo = jnp.where(tri, NEG, lo)
                    f_lo = NEG
                    f_hi = gather(hi, 0, 2)
                    x_hi = jnp.where(tri, NEG, gather(hi, 1, 2))
                for odd in range(2):
                    if odd == 0:
                        sm = jnp.concatenate([jnp.where(left64, x_lo, f_hi), jnp.where(left64, f_lo, x_hi)], axis=0)
                    else:
                        sm = jnp.concatenate([jnp.where(left64, f_hi, x_lo), jnp.where(left64, x_hi, f_lo)], axis=0)
                    m = jnp.max(sm, axis=0, keepdims=True)
                    s1 = None
                    if nk >= 2:
                        s1 = s_mid[:, 128 * (2 * t + odd):128 * (2 * t + odd + 1)]
                        m = jnp.maximum(m, jnp.max(s1, axis=0, keepdims=True))
                    res.append((sm, s1, m))
            return res

        def stage_pv(j, g, res):
            jb = i * NQ + j
            nk = nkeys(j)
            for t in range(4):
                hd = 4 * g + t
                odd = t % 2
                sm, s1, m = res[t]
                vw = lambda blk: _upk(vT_ref[blk, 16 * hd:16 * (hd + 1), :])
                pm = jnp.exp2(sm - m)
                p2 = jnp.where(uppers[odd], 0.0, pm) if nk == 3 else pm
                o = jnp.dot(vw(jb), p2.astype(bf16), preferred_element_type=f32)
                if nk == 3:
                    o = o + jnp.dot(vw(jb - 2), jnp.where(uppers[odd], pm, 0.0).astype(bf16), preferred_element_type=f32)
                if nk >= 2:
                    o = o + jnp.dot(vw(jb - 1), jnp.exp2(s1 - m).astype(bf16), preferred_element_type=f32)
                off = (20 * hd) % 16
                den = o[24:32] if off < 8 else o[0:8]
                rinv = 1.0 / den
                lo8 = off // 8 * 8
                on = o[lo8:lo8 + 24] * jnp.concatenate([rinv, rinv, rinv], axis=0)
                if odd:
                    on = pltpu.roll(on, 64, 1)
                oT_ref[20 * hd:20 * hd + 20, QB * j:QB * (j + 1)] = on[off - lo8:off - lo8 + 20]

        items = [(j, g) for j in range(NQ) for g in range(NG)]
        prev = stage_qk(*items[0])
        for n, it in enumerate(items[:-1]):
            nxt = stage_qk(*items[n + 1])
            stage_pv(*it, prev)
            prev = nxt
        return lambda: stage_pv(*items[-1], prev)

    def body(first, last):
        if not last:
            x_copy(i + 1).wait()
            hn = make_h(_ln(load_x(i + 1)))
        tail = attention(first)
        if not last:
            proj_k(hn, i + 1)
        tail()
        if not last:
            proj_q(hn)
        if first:
            cp_mod2.wait()
            mod_ref[:, 2 * D:] = jnp.dot(silu_c(), wmod_ref[:, 2 * D:], preferred_element_type=f32)
            cp_wo.wait()
        o_att = oT_ref[...].T.astype(bf16)
        attn = jnp.dot(o_att, wo_ref[...], preferred_element_type=f32)
        if first:
            cp_w1.wait()
            cp_w2.wait()
        if not last:
            proj_v(hn, i + 1)
        x1 = load_x(i) + modrow(2) * attn
        h2 = _ln(x1) * (1.0 + modrow(4)) + modrow(3)
        y = _ln(h2).astype(bf16)
        a = lax.dot_general(y, w1T_ref[...], NT, preferred_element_type=f32) + bias_ref[0:1, 0:F]
        gl = jax.nn.gelu(a, approximate=True).astype(bf16)
        mlp = jnp.dot(gl, w2_ref[...], preferred_element_type=f32) + bias_ref[1:2, 0:D]
        o_ref[...] = (x1 + modrow(5) * mlp).astype(o_ref.dtype)

    @pl.when(i == 0)
    def _():
        x_copy(0).start()
        cp_mod1.start()
        cp_wq.start()
        cp_wv.start()
        cp_wk.start()
        bias_ref[0:1, 0:F] = b1_ref[...].astype(f32).reshape(1, F)
        bias_ref[1:2, 0:D] = b2_ref[...].astype(f32).reshape(1, D)
        sc = silu_c()
        x_copy(0).wait()
        xn = _ln(load_x(0))
        cp_mod1.wait()
        x_copy(1).start()
        cp_mod2.start()
        cp_wo.start()
        cp_w1.start()
        cp_w2.start()
        for b in range(2, NB):
            x_copy(b).start()
        mod_ref[:, 0:2 * D] = jnp.dot(sc, wmod_ref[:, 0:2 * D], preferred_element_type=f32)
        h = make_h(xn)
        cp_wq.wait()
        proj_q(h)
        cp_wv.wait()
        wvT_ref[...] = _pk(wqkv_ref[:, 2 * D:3 * D].astype(f32).T)
        cp_wk.wait()
        proj_k(h, 0)
        proj_v(h, 0)
        body(True, False)

    @pl.when(jnp.logical_and(i > 0, i < NB - 1))
    def _():
        body(False, False)

    @pl.when(i == NB - 1)
    def _():
        body(False, True)


@jax.jit
def pallas_adaLN_cond__sliding_block__mixer_channel_mlp__prompt_kernel(
    A_x, A_wqkv, A_wo, B_x, B_w1, B_b1, B_w2, B_b2, c, w_mod,
):
    x2 = A_x.reshape(S, D)
    full = lambda shape: pl.BlockSpec(shape, lambda i: (0,) * len(shape))
    hbm = pl.BlockSpec(memory_space=pl.ANY)
    out = pl.pallas_call(
        _kernel,
        grid=(NB,),
        in_specs=[hbm, hbm, hbm, hbm, full((F,)), hbm, full((D,)), full((1, D)), hbm],
        out_specs=pl.BlockSpec((TM, D), lambda i: (i, 0)),
        out_shape=jax.ShapeDtypeStruct((S, D), A_x.dtype),
        scratch_shapes=[
            pltpu.VMEM((S, D), bf16),
            pltpu.VMEM((D, 3 * D), bf16),
            pltpu.VMEM((D, D), bf16),
            pltpu.VMEM((F, D), bf16),
            pltpu.VMEM((F, D), bf16),
            pltpu.VMEM((D, 6 * D), bf16),
            pltpu.VMEM((8, 6 * D), f32),
            pltpu.VMEM((8, F), f32),
            pltpu.VMEM((D // 2, D), u32),
            pltpu.VMEM((S // 2, NG * 128), u32),
            pltpu.VMEM((TM // 2, NG * 128), u32),
            pltpu.VMEM((S // QB, H * 16, QB), u32),
            pltpu.VMEM((D, TM), f32),
            pltpu.SemaphoreType.DMA((NB,)),
            pltpu.SemaphoreType.DMA((8,)),
        ],
        compiler_params=pltpu.CompilerParams(
            dimension_semantics=("arbitrary",),
            vmem_limit_bytes=100 * 1024 * 1024,
        ),
        name="adaln_kernel",
    )(x2, A_wqkv, A_wo, B_w1.T, B_b1, B_w2, B_b2, c, w_mod)
    return out.reshape(1, S, D)
```

```python
import functools
import math
import jax
import jax.numpy as jnp
from jax import lax
import jax.experimental.pallas as pl
import jax.experimental.pallas.tpu as pltpu

S = 2048
D = 640
H = 32
DH = 20
F = 1728
F1 = 896
TM = 256
NB = S // TM
QB = 128
NQ = TM // QB
NG = 8
EPS = 1e-5
QSCALE = (DH ** -0.5) * math.log2(math.e)
NEG = -1e30
LAG = 2
RCP = 1
EXS = 1
NSLOT = 4
f32 = jnp.float32
bf16 = jnp.bfloat16
u32 = jnp.uint32
NT = (((1,), (1,)), ((), ()))


def _pk(a):
    return pltpu.bitcast(a.astype(bf16), u32)


def _upk(a):
    return pltpu.bitcast(a, bf16)


def _ln(x):
    mu = jnp.mean(x, axis=-1, keepdims=True)
    xc = x - mu
    var = jnp.mean(xc * xc, axis=-1, keepdims=True)
    return xc * lax.rsqrt(var + EPS)


def _group_tiles(a):
    m = a.shape[0]
    lane = lax.broadcasted_iota(jnp.int32, (m, 128), 1)
    hi = lane >= 64
    t = [a[:, 128 * j:128 * (j + 1)] for j in range(5)]
    out = []
    for g in range(NG):
        lo_t, hi_t = (80 * g) // 128, (80 * g + 79) // 128
        out.append(t[lo_t] if lo_t == hi_t else jnp.where(hi, t[lo_t], t[hi_t]))
    return out


def _kernel(x_hbm, wqkv_hbm, wo_hbm, w1T_hbm, b1_hbm, w2_hbm, b2_hbm, c_hbm, wmod_hbm,
            o_hbm,
            x_ref, wqkv_ref, wo_ref, w1T_ref, w2_ref, wmod_ref, b1_ref, b2_ref, c_ref,
            mod_ref, bias_ref, wT_ref, k_ref, q_ref, vT_ref, oT_ref, y_ref, x1_ref, o_ref, s_ref, xsem, wsem, osem):
    i = pl.program_id(0)

    def x_copy(b):
        return pltpu.make_async_copy(x_hbm.at[pl.ds(b * TM, TM)], x_ref.at[pl.ds(b * TM, TM)], xsem.at[b])

    def o_copy(b):
        return pltpu.make_async_copy(o_ref.at[pl.ds(b * TM, TM)], o_hbm.at[pl.ds(b * TM, TM)], osem.at[b])

    def col_copy(src, dst, c0, n, s):
        return pltpu.make_async_copy(src.at[:, pl.ds(c0, n)], dst.at[:, pl.ds(c0, n)], wsem.at[s])

    cp_mod1 = col_copy(wmod_hbm, wmod_ref, 0, 2 * D, 0)
    cp_wq = col_copy(wqkv_hbm, wqkv_ref, 0, D, 1)
    cp_wk = col_copy(wqkv_hbm, wqkv_ref, D, D, 2)
    cp_wv = col_copy(wqkv_hbm, wqkv_ref, 2 * D, D, 3)
    cp_mod2 = col_copy(wmod_hbm, wmod_ref, 2 * D, 3 * D, 4)
    cp_mod3 = col_copy(wmod_hbm, wmod_ref, 5 * D, D, 5)
    cp_wo = pltpu.make_async_copy(wo_hbm, wo_ref, wsem.at[6])
    cp_w1 = pltpu.make_async_copy(w1T_hbm, w1T_ref, wsem.at[7])
    cp_w2 = pltpu.make_async_copy(w2_hbm, w2_ref, wsem.at[8])
    cp_b1 = pltpu.make_async_copy(b1_hbm, b1_ref, wsem.at[9])
    cp_b2 = pltpu.make_async_copy(b2_hbm, b2_ref, wsem.at[10])
    cp_c = pltpu.make_async_copy(c_hbm, c_ref, wsem.at[11])

    def modrow(k):
        return mod_ref[0:1, k * D:(k + 1) * D]

    def silu_c():
        c = c_ref[...].astype(f32)
        sc = c * jax.nn.sigmoid(c)
        return jnp.broadcast_to(sc, (8, D)).astype(bf16)

    def mod_cols(k0, k1):
        mod_ref[:, k0 * D:k1 * D] = jnp.dot(silu_c(), wmod_ref[:, k0 * D:k1 * D], preferred_element_type=f32)

    def load_x(b):
        return x_ref[pl.ds(pl.multiple_of(b * TM, TM), TM), :].astype(f32)

    def make_h(xn):
        return (xn * (1.0 + modrow(1)) + modrow(0)).astype(bf16)

    def store_q(qT):
        qTp = _pk(qT * QSCALE)
        r = lax.broadcasted_iota(jnp.int32, (40, QB), 0)
        oddrow = ((r >= 10) & (r < 20)) | (r >= 30)
        for j in range(NQ):
            for g in range(NG):
                blk = qTp[40 * g:40 * (g + 1), QB * j:QB * (j + 1)]
                q_ref[40 * g:40 * (g + 1), QB * j:QB * (j + 1)] = jnp.where(oddrow, pltpu.roll(blk, 64, 1), blk)

    def store_v(vT, b):
        vTp = _pk(vT)
        r16 = lax.broadcasted_iota(jnp.int32, (16, QB), 0)
        ones = jnp.full((16, QB), 0x3F803F80, u32)
        for hd in range(H):
            base = (10 * hd) // 8 * 8
            off = 10 * hd - base
            useful = (r16 >= off) & (r16 < off + 10)
            for j in range(NQ):
                win = vTp[base:base + 16, QB * j:QB * (j + 1)]
                vT_ref[b * NQ + j, 16 * hd:16 * (hd + 1), :] = jnp.where(useful, win, ones)

    def proj_q(h):
        store_q(lax.dot_general(_upk(wT_ref[0:D // 2, :]), h, NT, preferred_element_type=f32))

    def proj_v(h, b):
        store_v(lax.dot_general(_upk(wT_ref[D // 2:D, :]), h, NT, preferred_element_type=f32), b)

    def proj_k(h, b):
        k = jnp.dot(h, wqkv_ref[:, D:2 * D], preferred_element_type=f32)
        row0 = b * (TM // 2)
        kt = _group_tiles(_pk(k))
        for g in range(NG):
            k_ref[pl.ds(row0, TM // 2), 128 * g:128 * (g + 1)] = kt[g]

    def attention(blk, first):
        r64 = lax.broadcasted_iota(jnp.int32, (64, 128), 0)
        l64 = lax.broadcasted_iota(jnp.int32, (64, 128), 1)
        tri = r64 > (l64 & 63)
        left64 = l64 < 64
        r16 = lax.broadcasted_iota(jnp.int32, (16, 128), 0)
        left16 = lax.broadcasted_iota(jnp.int32, (16, 128), 1) < 64
        kj = lax.broadcasted_iota(jnp.int32, (QB, QB), 0)
        qi = lax.broadcasted_iota(jnp.int32, (QB, QB), 1)
        uppers = (kj > qi, kj > (qi ^ 64))

        def nkeys(j):
            return min(j + 1, 3) if first else 3

        def stage_qk(j, g):
            jb = blk * NQ + j
            nk = nkeys(j)
            cols = slice(128 * g, 128 * (g + 1))

            def krows(tile, a, n):
                st = (jb - 2 + tile) * 64 + a // 2
                return k_ref[st:st + n // 2, cols]

            qx = _upk(q_ref[40 * g:40 * (g + 1), QB * j:QB * (j + 1)]).astype(f32)

            def stat1(lh, rh):
                blocks = [None] * 8
                for k in range(5):
                    lo_r, hi_r = 16 * k, 16 * k + 16
                    def inter(hh):
                        return max(lo_r, 20 * hh) < min(hi_r, 20 * hh + 20)
                    if not (inter(lh) or inter(rh)):
                        continue
                    rr = r16 + lo_r
                    ml = (rr >= 20 * lh) & (rr < 20 * lh + 20)
                    if lh == rh:
                        msk = ml
                    else:
                        mr = (rr >= 20 * rh) & (rr < 20 * rh + 20)
                        msk = (ml & left16) | (mr & jnp.logical_not(left16))
                    blocks[(5 * g + k) % 8] = jnp.where(msk, qx[lo_r:hi_r], 0.0)
                z = jnp.zeros((16, 128), f32)
                return jnp.concatenate([z if b_ is None else b_ for b_ in blocks], axis=0)

            def stat(lst):
                return jnp.concatenate([stat1(lh, rh) for lh, rh in lst], axis=1).astype(bf16)

            p_lo, p_hi = [], []
            for c in range(4):
                if nk == 3:
                    p_lo += [krows(0, 16 * c, 16), krows(2, 16 * c, 16), krows(0, 64 + 16 * c, 16)]
                    p_hi += [krows(2, 16 * c, 16), krows(0, 64 + 16 * c, 16), krows(2, 64 + 16 * c, 16)]
                else:
                    p_lo += [krows(2, 16 * c, 16)]
                    p_hi += [krows(2, 16 * c, 16), krows(2, 64 + 16 * c, 16)]
            k_lo = _upk(jnp.concatenate(p_lo, axis=0))
            k_hi = _upk(jnp.concatenate(p_hi, axis=0))
            s_lh = []
            for t in range(2):
                s_lh.append(jnp.dot(k_lo, stat([(2 * t, 2 * t + 1)]), preferred_element_type=f32))
                s_lh.append(jnp.dot(k_hi, stat([(2 * t + 1, 2 * t)]), preferred_element_type=f32))
            if nk >= 2:
                q_mid = stat([(0, 0), (1, 1), (2, 2), (3, 3)])
                s_mid = jnp.dot(_upk(krows(1, 0, 128)), q_mid, preferred_element_type=f32)

            def gather(s, k, n):
                return jnp.concatenate([s[16 * (n * c + k):16 * (n * c + k) + 16] for c in range(4)], axis=0)

            res = []
            for t in range(2):
                lo, hi = s_lh[2 * t], s_lh[2 * t + 1]
                if nk == 3:
                    x_lo = jnp.where(tri, gather(lo, 0, 3), gather(lo, 1, 3))
                    f_lo = gather(lo, 2, 3)
                    f_hi = gather(hi, 0, 3)
                    x_hi = jnp.where(tri, gather(hi, 1, 3), gather(hi, 2, 3))
                else:
                    x_lo = jnp.where(tri, NEG, lo)
                    f_lo = NEG
                    f_hi = gather(hi, 0, 2)
                    x_hi = jnp.where(tri, NEG, gather(hi, 1, 2))
                for odd in range(2):
                    if odd == 0:
                        top, bot = jnp.where(left64, x_lo, f_hi), jnp.where(left64, f_lo, x_hi)
                    else:
                        top, bot = jnp.where(left64, f_hi, x_lo), jnp.where(left64, x_hi, f_lo)
                    sm = jnp.concatenate([top, bot], axis=0)
                    tb = jnp.maximum(top, bot)
                    m8 = None
                    for c in range(4):
                        mc = jnp.maximum(tb[16 * c:16 * c + 8], tb[16 * c + 8:16 * c + 16])
                        m8 = mc if m8 is None else jnp.maximum(m8, mc)
                    s1 = None
                    if nk >= 2:
                        s1 = s_mid[:, 128 * (2 * t + odd):128 * (2 * t + odd + 1)]
                        for c in range(8):
                            mc = jnp.maximum(s1[16 * c:16 * c + 8], s1[16 * c + 8:16 * c + 16])
                            m8 = jnp.maximum(m8, mc)
                    m = jnp.max(m8, axis=0, keepdims=True)
                    if EXS:
                        slot = ((j * NG + g) % NSLOT) * 4 + 2 * t + odd
                        s_ref[slot, 0:QB] = sm
                        if s1 is not None:
                            s_ref[slot, QB:2 * QB] = s1
                        res.append((slot, None, m))
                    else:
                        res.append((sm, s1, m))
            return res

        def stage_pv(j, g, res):
            jb = blk * NQ + j
            nk = nkeys(j)
            vw = lambda b_, hd: _upk(vT_ref[b_, 16 * hd:16 * (hd + 1), :])
            heads = range(4)
            if EXS:
                res = [(s_ref[r[0], 0:QB], s_ref[r[0], QB:2 * QB] if nk >= 2 else None, r[2]) for r in res]
            pm = [jnp.exp2(res[t][0] - res[t][2]) for t in heads]
            o = [jnp.dot(vw(jb, 4 * g + t), (jnp.where(uppers[t % 2], 0.0, pm[t]) if nk == 3 else pm[t]).astype(bf16),
                         preferred_element_type=f32) for t in heads]
            if nk == 3:
                o = [o[t] + jnp.dot(vw(jb - 2, 4 * g + t), jnp.where(uppers[t % 2], pm[t], 0.0).astype(bf16),
                                    preferred_element_type=f32) for t in heads]
            if nk >= 2:
                o = [o[t] + jnp.dot(vw(jb - 1, 4 * g + t), jnp.exp2(res[t][1] - res[t][2]).astype(bf16),
                                    preferred_element_type=f32) for t in heads]
            for t in heads:
                hd = 4 * g + t
                off = (20 * hd) % 16
                den = o[t][24:32] if off < 8 else o[t][0:8]
                if RCP == 0:
                    rinv = 1.0 / den
                else:
                    r0 = pl.reciprocal(den, approx=True)
                    rinv = r0 * (2.0 - den * r0)
                lo8 = off // 8 * 8
                on = o[t][lo8:lo8 + 24] * jnp.concatenate([rinv, rinv, rinv], axis=0)
                if t % 2:
                    on = pltpu.roll(on, 64, 1)
                oT_ref[20 * hd:20 * hd + 20, QB * j:QB * (j + 1)] = on[off - lo8:off - lo8 + 20]

        items = [(j, g) for j in range(NQ) for g in range(NG)]
        pend = []
        for it in items:
            pend.append((it, stage_qk(*it)))
            if len(pend) > LAG:
                it0, r0 = pend.pop(0)
                stage_pv(*it0, r0)

        def tail():
            for it0, r0 in pend:
                stage_pv(*it0, r0)
        return tail

    def mlp_up():
        a = lax.dot_general(_upk(y_ref[...]), w1T_ref[...], NT, preferred_element_type=f32)
        return jax.nn.gelu(a + bias_ref[0:1, 0:F], approximate=True).astype(bf16)

    def out_proj():
        o_att = oT_ref[...].T.astype(bf16)
        return jnp.dot(o_att, wo_ref[...], preferred_element_type=f32)

    def post_attn(attn, b):
        x1 = load_x(b) + modrow(2) * attn
        x1_ref[b % 2] = x1
        h2 = _ln(x1) * (1.0 + modrow(4)) + modrow(3)
        y_ref[...] = _pk(_ln(h2))

    def mlp_down(gl, b, c0, c1):
        mlp = jnp.dot(gl, w2_ref[:, c0:c1], preferred_element_type=f32)
        res = x1_ref[b % 2, :, c0:c1] + mod_ref[0:1, 5 * D + c0:5 * D + c1] * (mlp + bias_ref[1:2, c0:c1])
        o_ref[pl.ds(pl.multiple_of(b * TM, TM), TM), c0:c1] = res.astype(o_ref.dtype)

    @pl.when(i == 0)
    def _():
        for cp in (cp_c, x_copy(0), cp_mod1, cp_wk, cp_wq, cp_wv, x_copy(1), cp_mod2, cp_wo,
                   cp_b1, cp_b2, cp_mod3, cp_w1, x_copy(2), cp_w2):
            cp.start()
        for b in range(3, NB):
            x_copy(b).start()
        cp_c.wait()
        x_copy(0).wait()
        xn = _ln(load_x(0))
        cp_mod1.wait()
        mod_cols(0, 2)
        h = make_h(xn)
        cp_wk.wait()
        proj_k(h, 0)
        cp_wq.wait()
        q0 = jnp.dot(h, wqkv_ref[:, 0:D], preferred_element_type=f32)
        cp_wv.wait()
        x_copy(1).wait()
        v0 = jnp.dot(h, wqkv_ref[:, 2 * D:3 * D], preferred_element_type=f32)
        store_q(q0.T)
        hn = make_h(_ln(load_x(1)))
        proj_k(hn, 1)
        store_v(v0.T, 0)
        tail = attention(0, True)
        wT_ref[D // 2:D, :] = _pk(wqkv_ref[:, 2 * D:3 * D].astype(f32).T)
        wT_ref[0:D // 2, :] = _pk(wqkv_ref[:, 0:D].astype(f32).T)
        proj_v(hn, 1)
        tail()
        proj_q(hn)
        cp_mod2.wait()
        cp_wo.wait()
        cp_b1.wait()
        cp_b2.wait()
        cp_mod3.wait()
        mod_cols(2, 5)
        bias_ref[0:1, 0:F] = b1_ref[...].astype(f32).reshape(1, F)
        bias_ref[1:2, 0:D] = b2_ref[...].astype(f32).reshape(1, D)
        attn = out_proj()
        post_attn(attn, 0)
        tail = attention(1, False)
        mod_cols(5, 6)
        tail()
        cp_w1.wait()
        cp_w2.wait()

    @pl.when(jnp.logical_and(i > 0, i < NB - 1))
    def _():
        x_copy(i + 1).wait()
        gl = mlp_up()
        hn = make_h(_ln(load_x(i + 1)))
        attn = out_proj()
        k_ref[0:TM // 2, :] = k_ref[TM // 2:TM, :]
        vT_ref[0:NQ] = vT_ref[NQ:2 * NQ]
        proj_k(hn, 1)
        post_attn(attn, i)
        proj_q(hn)
        proj_v(hn, 1)
        tail = attention(1, False)
        mlp_down(gl, i - 1, 0, 256)
        tail()
        mlp_down(gl, i - 1, 256, D)
        o_copy(i - 1).start()

    @pl.when(i == NB - 1)
    def _():
        gl = mlp_up()
        attn = out_proj()
        mlp_down(gl, NB - 2, 0, D)
        post_attn(attn, NB - 1)
        o_copy(NB - 2).start()
        gl = mlp_up()
        mlp_down(gl, NB - 1, 0, D)
        o_copy(NB - 1).start()
        for b in range(NB):
            o_copy(b).wait()


@jax.jit
def pallas_adaLN_cond__sliding_block__mixer_channel_mlp__prompt_kernel(
    A_x, A_wqkv, A_wo, B_x, B_w1, B_b1, B_w2, B_b2, c, w_mod,
):
    x2 = A_x.reshape(S, D)
    hbm = pl.BlockSpec(memory_space=pl.ANY)
    out = pl.pallas_call(
        _kernel,
        grid=(NB,),
        in_specs=[hbm] * 9,
        out_specs=hbm,
        out_shape=jax.ShapeDtypeStruct((S, D), A_x.dtype),
        scratch_shapes=[
            pltpu.VMEM((S, D), bf16),
            pltpu.VMEM((D, 3 * D), bf16),
            pltpu.VMEM((D, D), bf16),
            pltpu.VMEM((F, D), bf16),
            pltpu.VMEM((F, D), bf16),
            pltpu.VMEM((D, 6 * D), bf16),
            pltpu.VMEM((F,), bf16),
            pltpu.VMEM((D,), bf16),
            pltpu.VMEM((1, D), bf16),
            pltpu.VMEM((8, 6 * D), f32),
            pltpu.VMEM((8, F), f32),
            pltpu.VMEM((D, D), u32),
            pltpu.VMEM((TM, NG * 128), u32),
            pltpu.VMEM((D // 2, TM), u32),
            pltpu.VMEM((2 * NQ, H * 16, QB), u32),
            pltpu.VMEM((D, TM), f32),
            pltpu.VMEM((TM // 2, D), u32),
            pltpu.VMEM((2, TM, D), f32),
            pltpu.VMEM((S, D), bf16),
            pltpu.VMEM((NSLOT * 4, 2 * QB, QB), f32),
            pltpu.SemaphoreType.DMA((NB,)),
            pltpu.SemaphoreType.DMA((12,)),
            pltpu.SemaphoreType.DMA((NB,)),
        ],
        compiler_params=pltpu.CompilerParams(
            dimension_semantics=("arbitrary",),
            vmem_limit_bytes=100 * 1024 * 1024,
        ),
        name="adaln_kernel",
    )(x2, A_wqkv, A_wo, B_w1.T, B_b1, B_w2, B_b2, c, w_mod)
    return out.reshape(1, S, D)
```

```python
import functools
import math

import jax
import jax.numpy as jnp
from jax import lax
import jax.experimental.pallas as pl
import jax.experimental.pallas.tpu as pltpu

S = 2048
D = 640
H = 32
DH = 20
F = 1728
FM = 1664
TM = 256
NB = S // TM
QB = 128
NQ = TM // QB
NG = 8
NSLOT = 5
EPS = 1e-5
QSCALE = (DH ** -0.5) * math.log2(math.e)
NEG = -1e30
f32 = jnp.float32
bf16 = jnp.bfloat16
u32 = jnp.uint32
NT = (((1,), (1,)), ((), ()))
NN = (((1,), (0,)), ((), ()))

S0V = 2
HB = 11
HW = 20
MC = 2
VM = 10
GB = 0
HS = 1
WQ = 4
KEEP = 1
LAG0 = 3
PVO0 = 0
JG0 = 1
CH0 = 32


def _pk(a):
    return pltpu.bitcast(a.astype(bf16), u32)


def _upk(a):
    return pltpu.bitcast(a, bf16)


def _mm(a, b, dims=NN):
    return lax.dot_general(a, b, dims, preferred_element_type=f32)


def _ln(x):
    mu = jnp.mean(x, axis=-1, keepdims=True)
    xc = x - mu
    var = jnp.mean(xc * xc, axis=-1, keepdims=True)
    return xc * lax.rsqrt(var + EPS)


def _group_tiles(a):
    lane = lax.broadcasted_iota(jnp.int32, (a.shape[0], 128), 1)
    t = [a[:, 128 * j:128 * (j + 1)] for j in range(5)]
    out = []
    for g in range(NG):
        lo_t, hi_t = (80 * g) // 128, (80 * g + 79) // 128
        out.append(t[lo_t] if lo_t == hi_t else jnp.where(lane >= 64, t[lo_t], t[hi_t]))
    return out


def _kernel(x_hbm, wqkv_hbm, wo_hbm, w1T_hbm, b1_hbm, w2_hbm, b2_hbm, c_hbm, wmod_hbm,
            o_hbm,
            x_ref, wqkv_ref, wo_ref, w1T_ref, w2_ref, wmod_ref, b1_ref, b2_ref, c_ref,
            sc_ref, mod_ref, bias_ref, wT_ref, k_ref, q_ref, vT_ref, oT_ref, y_ref, x1_ref, o_ref, s_ref, kf_ref,
            sem):
    i = pl.program_id(0)

    def x_copy(b, s, n=1):
        return pltpu.make_async_copy(x_hbm.at[pl.ds(b * TM, n * TM)], x_ref.at[pl.ds(b * TM, n * TM)], sem.at[s])

    def o_copy(b, c0=0, c1=D):
        return pltpu.make_async_copy(o_ref.at[pl.ds(b * TM, TM), pl.ds(c0, c1 - c0)],
                                     o_hbm.at[pl.ds(b * TM, TM), pl.ds(c0, c1 - c0)], sem.at[10])

    def col_copy(src, dst, c0, n, s):
        return pltpu.make_async_copy(src.at[:, pl.ds(c0, n)], dst.at[:, pl.ds(c0, n)], sem.at[s])

    cp_c = pltpu.make_async_copy(c_hbm, c_ref, sem.at[0])
    cp_x0 = x_copy(0, 0)
    cp_x1 = x_copy(1, 1)
    cp_ca = col_copy(wmod_hbm, wmod_ref, D, D, 2)
    cp_wk = col_copy(wqkv_hbm, wqkv_ref, D, D, 3)
    cp_wq = col_copy(wqkv_hbm, wqkv_ref, 0, D, 4)
    cp_sa = col_copy(wmod_hbm, wmod_ref, 0, D, 5)
    cp_wv = col_copy(wqkv_hbm, wqkv_ref, 2 * D, D, 6)
    cp_mid = (col_copy(wmod_hbm, wmod_ref, 2 * D, 4 * D, 7),
              pltpu.make_async_copy(wo_hbm, wo_ref, sem.at[7]),
              pltpu.make_async_copy(b1_hbm, b1_ref, sem.at[7]),
              pltpu.make_async_copy(b2_hbm, b2_ref, sem.at[7]))
    cp_late = (pltpu.make_async_copy(w1T_hbm, w1T_ref, sem.at[8]),
               pltpu.make_async_copy(w2_hbm, w2_ref, sem.at[8]),
               x_copy(2, 8))
    cp_xr = x_copy(3, 9, NB - 3)

    def modrow(k):
        return mod_ref[0:1, k * D:(k + 1) * D]

    def mod_span(c0, c1):
        mod_ref[:, c0:c1] = _mm(sc_ref[...], wmod_ref[:, c0:c1])

    def mod_cols(k0, k1):
        mod_span(k0 * D, k1 * D)

    def next_h(b, ch):
        hs = []
        for r0 in range(0, TM, ch):
            xc = x_ref[pl.ds(pl.multiple_of(b * TM + r0, ch), ch), :].astype(f32)
            hs.append(_ln(xc) * (1.0 + modrow(1)) + modrow(0))
        return jnp.concatenate(hs, axis=0).astype(bf16)

    def store_q(qT, b):
        qTp = _pk(qT * QSCALE)
        r8 = lax.broadcasted_iota(jnp.int32, (8, QB), 0)
        for j in range(NQ):
            for g in range(NG):
                for v in range(5):
                    rows = slice(40 * g + 8 * v, 40 * g + 8 * v + 8)
                    blk = qTp[rows, QB * j:QB * (j + 1)]
                    k0, k1 = (8 * v) // 10, (8 * v + 7) // 10
                    rl = lambda k: blk if k == 0 else pltpu.roll(blk, 32 * k, 1)
                    val = rl(k0) if k0 == k1 else jnp.where(r8 + 8 * v < 10 * k1, rl(k0), rl(k1))
                    q_ref[b * NQ + j, rows, :] = val

    def store_v(vT, b):
        r24 = lax.broadcasted_iota(jnp.int32, (24, QB), 0)
        for hd in range(H):
            base = (20 * hd) // 8 * 8
            off = 20 * hd - base
            useful = (r24 >= off) & (r24 < off + 20)
            for j in range(NQ):
                win = vT[base:base + 24, QB * j:QB * (j + 1)]
                vT_ref[b * NQ + j, 24 * hd:24 * (hd + 1), :] = jnp.where(useful, win, 1.0)

    def store_k(k, b):
        kt = _group_tiles(_pk(k))
        for g in range(NG):
            k_ref[b * (TM // 2):(b + 1) * (TM // 2), 128 * g:128 * (g + 1)] = kt[g]

    def proj_q(h, b):
        store_q(_mm(_upk(wT_ref[0:D // 2, :]), h, NT), b)

    def proj_v(h, b):
        store_v(_mm(_upk(wT_ref[D // 2:D, :]), h, NT), b)

    def proj_k(h, b):
        store_k(_mm(h, wqkv_ref[:, D:2 * D]), b)

    def attention(items, lag, pv_order, keep=None, hooks=None):
        r32 = lax.broadcasted_iota(jnp.int32, (32, 128), 0)
        l32 = lax.broadcasted_iota(jnp.int32, (32, 128), 1)
        tri = r32 > (l32 & 31)
        g_odd = (l32 & 32) != 0
        g_hi = l32 >= 64
        r16 = lax.broadcasted_iota(jnp.int32, (16, 128), 0)
        lg16 = lax.broadcasted_iota(jnp.int32, (16, 128), 1) >> 5
        kj = lax.broadcasted_iota(jnp.int32, (QB, QB), 0)
        qi = lax.broadcasted_iota(jnp.int32, (QB, QB), 1)
        uppers = [kj > ((qi - 32 * k) & 127) for k in range(4)]

        def stage_qk(n, jb, g):
            nk = min(jb + 1, 3)

            def krows(tile, a, cnt):
                st = (jb - 2 + tile) * 64 + a // 2
                return k_ref[st:st + cnt // 2, 128 * g:128 * (g + 1)]

            qx = _upk(q_ref[jb, 40 * g:40 * (g + 1), :]).astype(f32)

            def stat(heads, r):
                blocks = [None] * 8
                for v in range(5):
                    lo_r, hi_r = 16 * v, 16 * v + 16
                    msk = None
                    for k in heads:
                        if max(lo_r, 20 * k) >= min(hi_r, 20 * k + 20):
                            continue
                        rr = r16 + lo_r
                        mk = (rr >= 20 * k) & (rr < 20 * k + 20)
                        if r is not None:
                            mk = mk & (lg16 == (r + k) % 4)
                        msk = mk if msk is None else (msk | mk)
                    if msk is not None:
                        blocks[(5 * g + v) % 8] = jnp.where(msk, qx[lo_r:hi_r], 0.0)
                z = jnp.zeros((16, 128), f32)
                return jnp.concatenate([z if b_ is None else b_ for b_ in blocks], axis=0).astype(bf16)

            sq = [None] * 4
            for r in (range(4) if (nk == 3 or g % 2 == 0) else range(3, -1, -1)):
                parts, idx = [], []
                for c in range(4):
                    if c >= r and nk == 3:
                        parts.append(krows(0, 32 * c, 32))
                        idx.append((c, 0))
                    if c <= r:
                        parts.append(krows(2, 32 * c, 32))
                        idx.append((c, 2))
                s = _mm(_upk(jnp.concatenate(parts, axis=0)), stat(range(4), r))
                piece = {key: s[32 * m:32 * m + 32] for m, key in enumerate(idx)}
                neg = jnp.full((32, 128), NEG, f32)
                sq[r] = [piece[(c, 2)] if c < r else
                         (jnp.where(tri, piece.get((c, 0), neg), piece[(c, 2)]) if c == r else piece.get((c, 0), neg))
                         for c in range(4)]
            m8 = [None] * 4
            slot0 = (n % NSLOT) * 4
            for c in range(4):
                tt = [sq[(-k) % 4][c] for k in range(4)]
                uu = [jnp.where(g_odd, tt[(k - 1) % 4], tt[k]) for k in range(4)]
                for k in range(4):
                    sk = jnp.where(g_hi, uu[(k - 2) % 4], uu[k])
                    s_ref[slot0 + k, 32 * c:32 * c + 32] = sk
                    mc = jnp.maximum(jnp.maximum(sk[0:8], sk[8:16]), jnp.maximum(sk[16:24], sk[24:32]))
                    m8[k] = mc if m8[k] is None else jnp.maximum(m8[k], mc)
            yield None
            if nk >= 2:
                k1 = _upk(krows(1, 0, 128))
                s_mid = [_mm(k1, stat([k], None)) for k in range(4)]
            mx = []
            for k in range(4):
                if nk >= 2:
                    s1 = s_mid[k]
                    s_ref[slot0 + k, QB:2 * QB] = s1
                    for c in range(8):
                        m8[k] = jnp.maximum(m8[k], jnp.maximum(s1[16 * c:16 * c + 8], s1[16 * c + 8:16 * c + 16]))
                mx.append(jnp.max(m8[k], axis=0, keepdims=True))
            yield mx

        def stage_pv(n, jb, g, mx):
            nk = min(jb + 1, 3)
            slot0 = (n % NSLOT) * 4
            o = [None] * 4
            pm = [None] * 4

            def acc(k, tile, p):
                hd = 4 * g + k
                d = _mm(vT_ref[jb - 2 + tile, 24 * hd:24 * (hd + 1), :], p.astype(bf16))
                o[k] = d if o[k] is None else o[k] + d

            def merged(k):
                if pm[k] is None:
                    pm[k] = jnp.exp2(s_ref[slot0 + k, 0:QB] - mx[k])
                return pm[k]

            for tile in pv_order:
                for k in range(4):
                    if tile == 2:
                        acc(k, 2, jnp.where(uppers[k], 0.0, merged(k)) if nk == 3 else merged(k))
                    elif tile == 0 and nk == 3:
                        acc(k, 0, jnp.where(uppers[k], merged(k), 0.0))
                    elif tile == 1 and nk >= 2:
                        acc(k, 1, jnp.exp2(s_ref[slot0 + k, QB:2 * QB] - mx[k]))
                yield None
            for k in range(4):
                hd = 4 * g + k
                off = (20 * hd) % 8
                den = o[k][20:21] if off == 0 else o[k][0:1]
                r0 = pl.reciprocal(den, approx=True)
                on = o[k] * (r0 * (2.0 - den * r0))
                if k:
                    on = pltpu.roll(on, 128 - 32 * k, 1)
                oT_ref[20 * hd:20 * hd + 20, QB * jb:QB * (jb + 1)] = on[off:off + 20]

        def run_pv(args):
            for _ in stage_pv(*args):
                pass

        pend = []
        for n, it in enumerate(items):
            qk = stage_qk(n, *it)
            pv = stage_pv(*pend.pop(0)) if len(pend) >= lag else iter(())
            next(qk)
            next(pv, None)
            next(pv, None)
            pend.append((n, *it, next(qk)))
            for _ in pv:
                pass
            if keep is not None and len(pend) > keep + (len(items) - 1 - n) and len(pend) > 1:
                run_pv(pend.pop(0))
            if hooks and n in hooks:
                hooks[n]()
        return [functools.partial(run_pv, args) for args in pend]

    def block_items(blk, j_inner):
        if j_inner:
            return [(blk * NQ + j, g) for g in range(NG) for j in range(NQ)]
        return [(blk * NQ + j, g) for j in range(NQ) for g in range(NG)]

    def attn_rows(slot):
        return oT_ref[:, slot * TM:(slot + 1) * TM].T

    def post_attn(o_att, b, r0, r1, ch, mk=()):
        a = o_att[r0:r1].astype(bf16)
        if mk:
            outs = []
            for n in range(5):
                outs.append(_mm(a, wo_ref[:, 128 * n:128 * (n + 1)]))
                for m in mk:
                    mod_span(m * D + 128 * n, m * D + 128 * (n + 1))
            attn = jnp.concatenate(outs, axis=1)
        else:
            attn = _mm(a, wo_ref[...])
        xb = x_ref[pl.ds(pl.multiple_of(b * TM + r0, 16), r1 - r0), :].astype(f32)
        x1_ref[b % 2, r0:r1] = xb + modrow(2) * attn
        for c0 in range(r0, r1, ch):
            h2 = _ln(x1_ref[b % 2, c0:c0 + ch, :]) * (1.0 + modrow(4)) + modrow(3)
            y_ref[c0 // 2:(c0 + ch) // 2, :] = _pk(_ln(h2))

    def mlp_up(left_last):
        y = _upk(y_ref[...])
        if not left_last:
            alT = _mm(w1T_ref[FM:F, :], y, NT)
        am = _mm(y, w1T_ref[0:FM, :], NT)
        if left_last:
            alT = _mm(w1T_ref[FM:F, :], y, NT)
        a = jnp.concatenate([am, alT.T], axis=1)
        return jax.nn.gelu(a + bias_ref[0:1, 0:F], approximate=True).astype(bf16)

    def mlp_down(gl, b, c0, c1):
        mlp = _mm(gl, w2_ref[:, c0:c1])
        res = x1_ref[b % 2, :, c0:c1] + mod_ref[0:1, 5 * D + c0:5 * D + c1] * (mlp + bias_ref[1:2, c0:c1])
        o_ref[pl.ds(pl.multiple_of(b * TM, TM), TM), c0:c1] = res.astype(o_ref.dtype)

    @pl.when(i == 0)
    def _():
        for cp in (cp_c, cp_x0, cp_x1, cp_ca, cp_wk, cp_wq, cp_sa, cp_wv, *cp_mid, *cp_late, cp_xr):
            cp.start()
        cp_c.wait()
        cp_x0.wait()
        cf = c_ref[...].astype(f32)
        sc_ref[...] = jnp.broadcast_to(cf * jax.nn.sigmoid(cf), (8, D))
        x1_ref[0] = _ln(x_ref[0:TM, :].astype(f32))
        cp_x1.wait()
        x1_ref[1] = _ln(x_ref[TM:2 * TM, :].astype(f32))
        cp_ca.wait()
        mod_cols(1, 2)
        for b in range(2):
            x1_ref[b] = x1_ref[b] * (1.0 + modrow(1))

        def k_part(b):
            for r0 in range(0, TM, 64):
                kf_ref[b, r0:r0 + 64] = _mm(x1_ref[b, r0:r0 + 64].astype(bf16), wqkv_ref[:, D:2 * D])

        cp_wk.wait()
        k_part(0)
        cp_wq.wait()
        wT_ref[0:D // 2, :] = _pk(wqkv_ref[:, 0:D].astype(f32).T)
        k_part(1)
        cp_sa.wait()
        mod_cols(0, 1)
        h = (x1_ref[0] + modrow(0)).astype(bf16)
        hn = (x1_ref[1] + modrow(0)).astype(bf16)
        store_q(jnp.concatenate([_mm(_upk(wT_ref[r0:r0 + D // 4, :]), h, NT) for r0 in (0, D // 4)], axis=0), 0)
        kb = _mm(mod_ref[:, 0:D], wqkv_ref[:, D:2 * D])[0:1]
        cp_wv.wait()
        wT_ref[D // 2:D, :] = _pk(wqkv_ref[:, 2 * D:3 * D].astype(f32).T)
        store_k(kf_ref[0] + kb, 0)
        store_k(kf_ref[1] + kb, 1)
        proj_q(hn, 1)
        proj_v(h, 0)
        pvo = ((2, 0, 1), (1, 2, 0), (2, 1, 0))[PVO0]

        def wait_mid():
            for cp in cp_mid:
                cp.wait()
            bias_ref[0:1, 0:F] = b1_ref[...].astype(f32).reshape(1, F)
            bias_ref[1:2, 0:D] = b2_ref[...].astype(f32).reshape(1, D)

        if S0V == 0:
            for t in attention(block_items(0, JG0), LAG0, pvo, 1):
                t()
            wait_mid()
            mod_cols(2, 4)
            post_attn(attn_rows(0), 0, 0, TM, CH0, (4, 5))
            proj_v(hn, 1)
            for t in attention(block_items(1, JG0), LAG0, pvo, KEEP):
                t()
        else:
            hooks = {}

            def add(n, fn):
                prev = hooks.get(n)
                hooks[n] = fn if prev is None else (lambda: (prev(), fn()))

            def mod_chunk(m):
                mod_span(2 * D + 128 * m, 2 * D + 128 * (m + 1))

            def v1_with_mod():
                hf = x1_ref[1] + modrow(0)
                hj = [hf[QB * j:QB * (j + 1)].astype(bf16) for j in range(NQ)]
                rows, m = [], 0
                for r0 in range(0, D // 2, 64):
                    cols = []
                    for j in range(NQ):
                        cols.append(_mm(_upk(wT_ref[D // 2 + r0:D // 2 + r0 + 64, :]), hj[j], NT))
                        for _ in range(1 if VM == 10 or (VM == 15 and j == 0) else 2):
                            mod_chunk(m)
                            m += 1
                    rows.append(jnp.concatenate(cols, axis=1))
                store_v(jnp.concatenate(rows, axis=0), 1)

            add(HB, wait_mid)
            if S0V == 3:
                add(HB, v1_with_mod)
                first = VM
            else:
                proj_v(hn, 1)
                first = 0
            last_ = 15 if GB else 20
            for m in range(first, last_):
                add(HB + (S0V == 3) + (m - first) // MC, functools.partial(mod_chunk, m))
            hw = max(HW, HB + (S0V == 3) + max(14 - first, 0) // MC)
            for q_ in range(WQ):
                add(hw + HS * q_, functools.partial(
                    lambda q: post_attn(attn_rows(0), 0, q * TM // WQ, (q + 1) * TM // WQ, CH0), q_))
            tail = attention(block_items(0, JG0) + block_items(1, JG0), LAG0, pvo, KEEP, hooks)
            if GB and first < 20:
                mod_cols(5, 6)
            for t in tail:
                t()
        for cp in cp_late:
            cp.wait()

    @pl.when(i == 2)
    def _():
        cp_xr.wait()

    @pl.when(jnp.logical_and(i > 0, i < NB - 1))
    def _():
        k_ref[0:TM // 2, :] = k_ref[TM // 2:TM, :]
        vT_ref[0:NQ] = vT_ref[NQ:2 * NQ]
        gl = mlp_up(False)
        hn = next_h(i + 1, 32)
        o_att = attn_rows(1)
        proj_q(hn, 1)
        post_attn(o_att, i, 0, TM // 2, 64)
        proj_v(hn, 1)
        post_attn(o_att, i, TM // 2, TM, 64)
        proj_k(hn, 1)
        tail = attention(block_items(1, False), 3, (2, 1, 0))
        for n in range(5):
            if n < len(tail):
                tail[n]()
            mlp_down(gl, i - 1, 128 * n, 128 * (n + 1))
        o_copy(i - 1).start()

    @pl.when(i == NB - 1)
    def _():
        gl = mlp_up(True)
        o_att = attn_rows(1)
        for n in range(5):
            if n < 4:
                post_attn(o_att, NB - 1, 64 * n, 64 * (n + 1), 64)
            mlp_down(gl, NB - 2, 128 * n, 128 * (n + 1))
        o_copy(NB - 2).start()
        gl = mlp_up(True)
        chunks = ((0, 256), (256, 512), (512, D))
        for c0, c1 in chunks:
            mlp_down(gl, NB - 1, c0, c1)
            o_copy(NB - 1, c0, c1).start()
        for b in range(NB - 1):
            o_copy(b).wait()
        for c0, c1 in chunks:
            o_copy(NB - 1, c0, c1).wait()


@jax.jit
def pallas_adaLN_cond__sliding_block__mixer_channel_mlp__prompt_kernel(
    A_x: jax.Array,
    A_wqkv: jax.Array,
    A_wo: jax.Array,
    B_x: jax.Array,
    B_w1: jax.Array,
    B_b1: jax.Array,
    B_w2: jax.Array,
    B_b2: jax.Array,
    c: jax.Array,
    w_mod: jax.Array,
):
    del B_x
    hbm = pl.BlockSpec(memory_space=pl.ANY)
    out = pl.pallas_call(
        _kernel,
        grid=(NB,),
        in_specs=[hbm] * 9,
        out_specs=hbm,
        out_shape=jax.ShapeDtypeStruct((S, D), A_x.dtype),
        scratch_shapes=[
            pltpu.VMEM((S, D), bf16),
            pltpu.VMEM((D, 3 * D), bf16),
            pltpu.VMEM((D, D), bf16),
            pltpu.VMEM((F, D), bf16),
            pltpu.VMEM((F, D), bf16),
            pltpu.VMEM((D, 6 * D), bf16),
            pltpu.VMEM((F,), bf16),
            pltpu.VMEM((D,), bf16),
            pltpu.VMEM((1, D), bf16),
            pltpu.VMEM((8, D), f32),
            pltpu.VMEM((8, 6 * D), f32),
            pltpu.VMEM((8, F), f32),
            pltpu.VMEM((D, D), u32),
            pltpu.VMEM((TM, NG * 128), u32),
            pltpu.VMEM((2 * NQ, D // 2, QB), u32),
            pltpu.VMEM((2 * NQ, H * 24, QB), f32),
            pltpu.VMEM((D, 2 * TM), f32),
            pltpu.VMEM((TM // 2, D), u32),
            pltpu.VMEM((2, TM, D), f32),
            pltpu.VMEM((S, D), bf16),
            pltpu.VMEM((NSLOT * 4, 2 * QB, QB), f32),
            pltpu.VMEM((2, TM, D), f32),
            pltpu.SemaphoreType.DMA((11,)),
        ],
        compiler_params=pltpu.CompilerParams(
            dimension_semantics=("arbitrary",),
            vmem_limit_bytes=100 * 1024 * 1024,
        ),
        name="adaln_kernel",
    )(A_x.reshape(S, D), A_wqkv, A_wo, B_w1.T, B_b1, B_w2, B_b2, c, w_mod)
    return out.reshape(1, S, D)
```

```python
import functools
import math

import jax
import jax.numpy as jnp
from jax import lax
import jax.experimental.pallas as pl
import jax.experimental.pallas.tpu as pltpu

S = 2048
D = 640
H = 32
DH = 20
F = 1728
FM = 1664
TM = 256
NB = S // TM
QB = 128
NQ = TM // QB
NG = 8
NSLOT = 5
EPS = 1e-5
QSCALE = (DH ** -0.5) * math.log2(math.e)
NEG = -1e30
f32 = jnp.float32
bf16 = jnp.bfloat16
u32 = jnp.uint32
NT = (((1,), (1,)), ((), ()))
NN = (((1,), (0,)), ((), ()))


def _pk(a):
    return pltpu.bitcast(a.astype(bf16), u32)


def _upk(a):
    return pltpu.bitcast(a, bf16)


def _mm(a, b, dims=NN):
    return lax.dot_general(a, b, dims, preferred_element_type=f32)


def _ln(x):
    mu = jnp.mean(x, axis=-1, keepdims=True)
    xc = x - mu
    var = jnp.mean(xc * xc, axis=-1, keepdims=True)
    return xc * lax.rsqrt(var + EPS)


def _group_tiles(a):
    lane = lax.broadcasted_iota(jnp.int32, (a.shape[0], 128), 1)
    t = [a[:, 128 * j:128 * (j + 1)] for j in range(5)]
    out = []
    for g in range(NG):
        lo_t, hi_t = (80 * g) // 128, (80 * g + 79) // 128
        out.append(t[lo_t] if lo_t == hi_t else jnp.where(lane >= 64, t[lo_t], t[hi_t]))
    return out


def _kernel(x_hbm, wqkv_hbm, wo_hbm, w1T_hbm, b1_hbm, w2_hbm, b2_hbm, c_hbm, wmod_hbm,
            o_hbm,
            x_ref, wqkv_ref, wo_ref, w1T_ref, w2_ref, wmod_ref, b1_ref, b2_ref, c_ref,
            sc_ref, mod_ref, bias_ref, wT_ref, k_ref, q_ref, vT_ref, oT_ref, y_ref, x1_ref, o_ref, s_ref, kf_ref,
            sem):
    i = pl.program_id(0)

    def x_copy(b, s, n=1):
        return pltpu.make_async_copy(x_hbm.at[pl.ds(b * TM, n * TM)], x_ref.at[pl.ds(b * TM, n * TM)], sem.at[s])

    def o_copy(b, c0=0, c1=D):
        return pltpu.make_async_copy(o_ref.at[pl.ds(b * TM, TM), pl.ds(c0, c1 - c0)],
                                     o_hbm.at[pl.ds(b * TM, TM), pl.ds(c0, c1 - c0)], sem.at[2])

    def col_copy(src, dst, c0, n, s):
        return pltpu.make_async_copy(src.at[:, pl.ds(c0, n)], dst.at[:, pl.ds(c0, n)], sem.at[s])

    cp_first = (pltpu.make_async_copy(c_hbm, c_ref, sem.at[0]), x_copy(0, 0, 2))
    cp_ca = col_copy(wmod_hbm, wmod_ref, D, D, 1)
    cp_wk = col_copy(wqkv_hbm, wqkv_ref, D, D, 2)
    cp_q = (col_copy(wqkv_hbm, wqkv_ref, 0, D, 3), col_copy(wmod_hbm, wmod_ref, 0, D, 3))
    cp_wv = col_copy(wqkv_hbm, wqkv_ref, 2 * D, D, 4)
    cp_mid = (col_copy(wmod_hbm, wmod_ref, 2 * D, 4 * D, 5),
              pltpu.make_async_copy(wo_hbm, wo_ref, sem.at[5]),
              pltpu.make_async_copy(b1_hbm, b1_ref, sem.at[5]),
              pltpu.make_async_copy(b2_hbm, b2_ref, sem.at[5]))
    cp_late = (pltpu.make_async_copy(w1T_hbm, w1T_ref, sem.at[0]),
               pltpu.make_async_copy(w2_hbm, w2_ref, sem.at[0]),
               x_copy(2, 0))
    cp_xr = x_copy(3, 1, NB - 3)

    def modrow(k):
        return mod_ref[0:1, k * D:(k + 1) * D]

    def mod_span(c0, c1):
        mod_ref[:, c0:c1] = _mm(sc_ref[...], wmod_ref[:, c0:c1])

    def mod_cols(k0, k1):
        mod_span(k0 * D, k1 * D)

    def next_h(b, ch):
        hs = []
        for r0 in range(0, TM, ch):
            xc = x_ref[pl.ds(pl.multiple_of(b * TM + r0, ch), ch), :].astype(f32)
            hs.append(_ln(xc) * (1.0 + modrow(1)) + modrow(0))
        return jnp.concatenate(hs, axis=0).astype(bf16)

    def store_q(qT, b):
        qTp = _pk(qT * QSCALE)
        r8 = lax.broadcasted_iota(jnp.int32, (8, QB), 0)
        for j in range(NQ):
            for g in range(NG):
                for v in range(5):
                    rows = slice(40 * g + 8 * v, 40 * g + 8 * v + 8)
                    blk = qTp[rows, QB * j:QB * (j + 1)]
                    k0, k1 = (8 * v) // 10, (8 * v + 7) // 10
                    rl = lambda k: blk if k == 0 else pltpu.roll(blk, 32 * k, 1)
                    val = rl(k0) if k0 == k1 else jnp.where(r8 + 8 * v < 10 * k1, rl(k0), rl(k1))
                    q_ref[b * NQ + j, rows, :] = val

    def store_v(vT, b):
        r24 = lax.broadcasted_iota(jnp.int32, (24, QB), 0)
        for hd in range(H):
            base = (20 * hd) // 8 * 8
            off = 20 * hd - base
            useful = (r24 >= off) & (r24 < off + 20)
            for j in range(NQ):
                win = vT[base:base + 24, QB * j:QB * (j + 1)]
                vT_ref[b * NQ + j, 24 * hd:24 * (hd + 1), :] = jnp.where(useful, win, 1.0)

    def store_k(k, b):
        kt = _group_tiles(_pk(k))
        for g in range(NG):
            k_ref[b * (TM // 2):(b + 1) * (TM // 2), 128 * g:128 * (g + 1)] = kt[g]

    def proj_q(h, b):
        store_q(_mm(_upk(wT_ref[0:D // 2, :]), h, NT), b)

    def proj_v(h, b):
        store_v(_mm(_upk(wT_ref[D // 2:D, :]), h, NT), b)

    def proj_k(h, b):
        store_k(_mm(h, wqkv_ref[:, D:2 * D]), b)

    def attention(items, lag, pv_order, keep=None, hook=None):
        r32 = lax.broadcasted_iota(jnp.int32, (32, 128), 0)
        l32 = lax.broadcasted_iota(jnp.int32, (32, 128), 1)
        tri = r32 > (l32 & 31)
        g_odd = (l32 & 32) != 0
        g_hi = l32 >= 64
        r16 = lax.broadcasted_iota(jnp.int32, (16, 128), 0)
        lg16 = lax.broadcasted_iota(jnp.int32, (16, 128), 1) >> 5
        kj = lax.broadcasted_iota(jnp.int32, (QB, QB), 0)
        qi = lax.broadcasted_iota(jnp.int32, (QB, QB), 1)
        uppers = [kj > ((qi - 32 * k) & 127) for k in range(4)]

        def stage_qk(n, jb, g):
            nk = min(jb + 1, 3)

            def krows(tile, a, cnt):
                st = (jb - 2 + tile) * 64 + a // 2
                return k_ref[st:st + cnt // 2, 128 * g:128 * (g + 1)]

            qx = _upk(q_ref[jb, 40 * g:40 * (g + 1), :]).astype(f32)

            def stat(heads, r):
                blocks = [None] * 8
                for v in range(5):
                    lo_r, hi_r = 16 * v, 16 * v + 16
                    msk = None
                    for k in heads:
                        if max(lo_r, 20 * k) >= min(hi_r, 20 * k + 20):
                            continue
                        rr = r16 + lo_r
                        mk = (rr >= 20 * k) & (rr < 20 * k + 20)
                        if r is not None:
                            mk = mk & (lg16 == (r + k) % 4)
                        msk = mk if msk is None else (msk | mk)
                    if msk is not None:
                        blocks[(5 * g + v) % 8] = jnp.where(msk, qx[lo_r:hi_r], 0.0)
                z = jnp.zeros((16, 128), f32)
                return jnp.concatenate([z if b_ is None else b_ for b_ in blocks], axis=0).astype(bf16)

            sq = [None] * 4
            for r in (range(4) if (nk == 3 or g % 2 == 0) else range(3, -1, -1)):
                parts, idx = [], []
                for c in range(4):
                    if c >= r and nk == 3:
                        parts.append(krows(0, 32 * c, 32))
                        idx.append((c, 0))
                    if c <= r:
                        parts.append(krows(2, 32 * c, 32))
                        idx.append((c, 2))
                s = _mm(_upk(jnp.concatenate(parts, axis=0)), stat(range(4), r))
                piece = {key: s[32 * m:32 * m + 32] for m, key in enumerate(idx)}
                neg = jnp.full((32, 128), NEG, f32)
                sq[r] = [piece[(c, 2)] if c < r else
                         (jnp.where(tri, piece.get((c, 0), neg), piece[(c, 2)]) if c == r else piece.get((c, 0), neg))
                         for c in range(4)]
            m8 = [None] * 4
            slot0 = (n % NSLOT) * 4
            for c in range(4):
                tt = [sq[(-k) % 4][c] for k in range(4)]
                uu = [jnp.where(g_odd, tt[(k - 1) % 4], tt[k]) for k in range(4)]
                for k in range(4):
                    sk = jnp.where(g_hi, uu[(k - 2) % 4], uu[k])
                    s_ref[slot0 + k, 32 * c:32 * c + 32] = sk
                    mc = jnp.maximum(jnp.maximum(sk[0:8], sk[8:16]), jnp.maximum(sk[16:24], sk[24:32]))
                    m8[k] = mc if m8[k] is None else jnp.maximum(m8[k], mc)
            yield None
            if nk >= 2:
                k1 = _upk(krows(1, 0, 128))
                s_mid = [_mm(k1, stat([k], None)) for k in range(4)]
            mx = []
            for k in range(4):
                if nk >= 2:
                    s1 = s_mid[k]
                    s_ref[slot0 + k, QB:2 * QB] = s1
                    for c in range(8):
                        m8[k] = jnp.maximum(m8[k], jnp.maximum(s1[16 * c:16 * c + 8], s1[16 * c + 8:16 * c + 16]))
                mx.append(jnp.max(m8[k], axis=0, keepdims=True))
            yield mx

        def stage_pv(n, jb, g, mx):
            nk = min(jb + 1, 3)
            slot0 = (n % NSLOT) * 4
            o = [None] * 4
            pm = [None] * 4

            def acc(k, tile, p):
                hd = 4 * g + k
                d = _mm(vT_ref[jb - 2 + tile, 24 * hd:24 * (hd + 1), :], p.astype(bf16))
                o[k] = d if o[k] is None else o[k] + d

            def merged(k):
                if pm[k] is None:
                    pm[k] = jnp.exp2(s_ref[slot0 + k, 0:QB] - mx[k])
                return pm[k]

            for tile in pv_order:
                for k in range(4):
                    if tile == 2:
                        acc(k, 2, jnp.where(uppers[k], 0.0, merged(k)) if nk == 3 else merged(k))
                    elif tile == 0 and nk == 3:
                        acc(k, 0, jnp.where(uppers[k], merged(k), 0.0))
                    elif tile == 1 and nk >= 2:
                        acc(k, 1, jnp.exp2(s_ref[slot0 + k, QB:2 * QB] - mx[k]))
                yield None
            for k in range(4):
                hd = 4 * g + k
                off = (20 * hd) % 8
                den = o[k][20:21] if off == 0 else o[k][0:1]
                r0 = pl.reciprocal(den, approx=True)
                on = o[k] * (r0 * (2.0 - den * r0))
                if k:
                    on = pltpu.roll(on, 128 - 32 * k, 1)
                oT_ref[20 * hd:20 * hd + 20, QB * jb:QB * (jb + 1)] = on[off:off + 20]

        def run_pv(args):
            for _ in stage_pv(*args):
                pass

        pend = []
        for n, it in enumerate(items):
            qk = stage_qk(n, *it)
            pv = stage_pv(*pend.pop(0)) if len(pend) >= lag else iter(())
            next(qk)
            next(pv, None)
            next(pv, None)
            pend.append((n, *it, next(qk)))
            for _ in pv:
                pass
            if keep is not None and len(pend) > keep + (len(items) - 1 - n) and len(pend) > 1:
                run_pv(pend.pop(0))
            if hook is not None:
                hook(n)
        return [functools.partial(run_pv, args) for args in pend]

    def block_items(blk, j_inner):
        if j_inner:
            return [(blk * NQ + j, g) for g in range(NG) for j in range(NQ)]
        return [(blk * NQ + j, g) for j in range(NQ) for g in range(NG)]

    def attn_rows(slot):
        return oT_ref[:, slot * TM:(slot + 1) * TM].T

    def post_attn(o_att, b, r0, r1, ch):
        attn = _mm(o_att[r0:r1].astype(bf16), wo_ref[...])
        xb = x_ref[pl.ds(pl.multiple_of(b * TM + r0, 16), r1 - r0), :].astype(f32)
        x1_ref[b % 2, r0:r1] = xb + modrow(2) * attn
        for c0 in range(r0, r1, ch):
            h2 = _ln(x1_ref[b % 2, c0:c0 + ch, :]) * (1.0 + modrow(4)) + modrow(3)
            y_ref[c0 // 2:(c0 + ch) // 2, :] = _pk(_ln(h2))

    def mlp_up(left_last):
        y = _upk(y_ref[...])
        if not left_last:
            alT = _mm(w1T_ref[FM:F, :], y, NT)
        am = _mm(y, w1T_ref[0:FM, :], NT)
        if left_last:
            alT = _mm(w1T_ref[FM:F, :], y, NT)
        a = jnp.concatenate([am, alT.T], axis=1)
        return jax.nn.gelu(a + bias_ref[0:1, 0:F], approximate=True).astype(bf16)

    def mlp_down(gl, b, c0, c1):
        mlp = _mm(gl, w2_ref[:, c0:c1])
        res = x1_ref[b % 2, :, c0:c1] + mod_ref[0:1, 5 * D + c0:5 * D + c1] * (mlp + bias_ref[1:2, c0:c1])
        o_ref[pl.ds(pl.multiple_of(b * TM, TM), TM), c0:c1] = res.astype(o_ref.dtype)

    @pl.when(i == 0)
    def _():
        for cp in (*cp_first, cp_ca, cp_wk, *cp_q, cp_wv, *cp_mid):
            cp.start()
        for cp in cp_first:
            cp.wait()
        for cp in cp_late:
            cp.start()
        cf = c_ref[...].astype(f32)
        sc_ref[...] = jnp.broadcast_to(cf * jax.nn.sigmoid(cf), (8, D))
        for b in range(2):
            x1_ref[b] = _ln(x_ref[b * TM:(b + 1) * TM, :].astype(f32))
        cp_ca.wait()
        cp_xr.start()
        mod_cols(1, 2)
        for b in range(2):
            x1_ref[b] = x1_ref[b] * (1.0 + modrow(1))

        cp_wk.wait()
        for b in range(2):
            for r0 in range(0, TM, 64):
                kf_ref[b, r0:r0 + 64] = _mm(x1_ref[b, r0:r0 + 64].astype(bf16), wqkv_ref[:, D:2 * D])
        for cp in cp_q:
            cp.wait()
        mod_cols(0, 1)
        wT_ref[0:D // 2, :] = _pk(wqkv_ref[:, 0:D].astype(f32).T)
        h = (x1_ref[0] + modrow(0)).astype(bf16)
        hn = (x1_ref[1] + modrow(0)).astype(bf16)
        q0T = jnp.concatenate([_mm(_upk(wT_ref[r0:r0 + D // 4, :]), h, NT) for r0 in (0, D // 4)], axis=0)
        kb = _mm(mod_ref[:, 0:D], wqkv_ref[:, D:2 * D])[0:1]
        cp_wv.wait()
        store_q(q0T, 0)
        wT_ref[D // 2:D, :] = _pk(wqkv_ref[:, 2 * D:3 * D].astype(f32).T)
        store_k(kf_ref[0] + kb, 0)
        store_k(kf_ref[1] + kb, 1)
        proj_q(hn, 1)
        proj_v(h, 0)
        proj_v(hn, 1)

        def wait_mid():
            for cp in cp_mid:
                cp.wait()
            bias_ref[0:1, 0:F] = b1_ref[...].astype(f32).reshape(1, F)
            bias_ref[1:2, 0:D] = b2_ref[...].astype(f32).reshape(1, D)

        def hook(n):
            if n == 13:
                wait_mid()
            if 13 <= n < 23:
                for m in (2 * (n - 13), 2 * (n - 13) + 1):
                    mod_span(2 * D + 128 * m, 2 * D + 128 * (m + 1))
            if 21 <= n < 25:
                post_attn(attn_rows(0), 0, 64 * (n - 21), 64 * (n - 20), 32)

        for t in attention(block_items(0, True) + block_items(1, True), 3, (2, 0, 1), 1, hook):
            t()
        for cp in cp_late:
            cp.wait()

    @pl.when(i == 2)
    def _():
        cp_xr.wait()

    @pl.when(jnp.logical_and(i > 0, i < NB - 1))
    def _():
        k_ref[0:TM // 2, :] = k_ref[TM // 2:TM, :]
        vT_ref[0:NQ] = vT_ref[NQ:2 * NQ]
        gl = mlp_up(False)
        hn = next_h(i + 1, 32)
        o_att = attn_rows(1)
        proj_q(hn, 1)
        post_attn(o_att, i, 0, TM // 2, 64)
        proj_v(hn, 1)
        post_attn(o_att, i, TM // 2, TM, 64)
        proj_k(hn, 1)
        tail = attention(block_items(1, False), 3, (2, 1, 0))
        for n in range(5):
            if n < len(tail):
                tail[n]()
            mlp_down(gl, i - 1, 128 * n, 128 * (n + 1))
        o_copy(i - 1).start()

    @pl.when(i == NB - 1)
    def _():
        gl = mlp_up(True)
        o_att = attn_rows(1)
        for n in range(5):
            if n < 4:
                post_attn(o_att, NB - 1, 64 * n, 64 * (n + 1), 64)
            mlp_down(gl, NB - 2, 128 * n, 128 * (n + 1))
        o_copy(NB - 2).start()
        gl = mlp_up(True)
        chunks = ((0, 256), (256, 512), (512, D))
        for c0, c1 in chunks:
            mlp_down(gl, NB - 1, c0, c1)
            o_copy(NB - 1, c0, c1).start()
        for b in range(NB - 1):
            o_copy(b).wait()
        for c0, c1 in chunks:
            o_copy(NB - 1, c0, c1).wait()


@jax.jit
def pallas_adaLN_cond__sliding_block__mixer_channel_mlp__prompt_kernel(
    A_x: jax.Array,
    A_wqkv: jax.Array,
    A_wo: jax.Array,
    B_x: jax.Array,
    B_w1: jax.Array,
    B_b1: jax.Array,
    B_w2: jax.Array,
    B_b2: jax.Array,
    c: jax.Array,
    w_mod: jax.Array,
):
    del B_x
    hbm = pl.BlockSpec(memory_space=pl.ANY)
    out = pl.pallas_call(
        _kernel,
        grid=(NB,),
        in_specs=[hbm] * 9,
        out_specs=hbm,
        out_shape=jax.ShapeDtypeStruct((S, D), A_x.dtype),
        scratch_shapes=[
            pltpu.VMEM((S, D), bf16),
            pltpu.VMEM((D, 3 * D), bf16),
            pltpu.VMEM((D, D), bf16),
            pltpu.VMEM((F, D), bf16),
            pltpu.VMEM((F, D), bf16),
            pltpu.VMEM((D, 6 * D), bf16),
            pltpu.VMEM((F,), bf16),
            pltpu.VMEM((D,), bf16),
            pltpu.VMEM((1, D), bf16),
            pltpu.VMEM((8, D), f32),
            pltpu.VMEM((8, 6 * D), f32),
            pltpu.VMEM((8, F), f32),
            pltpu.VMEM((D, D), u32),
            pltpu.VMEM((TM, NG * 128), u32),
            pltpu.VMEM((2 * NQ, D // 2, QB), u32),
            pltpu.VMEM((2 * NQ, H * 24, QB), f32),
            pltpu.VMEM((D, 2 * TM), f32),
            pltpu.VMEM((TM // 2, D), u32),
            pltpu.VMEM((2, TM, D), f32),
            pltpu.VMEM((S, D), bf16),
            pltpu.VMEM((NSLOT * 4, 2 * QB, QB), f32),
            pltpu.VMEM((2, TM, D), f32),
            pltpu.SemaphoreType.DMA((6,)),
        ],
        compiler_params=pltpu.CompilerParams(
            dimension_semantics=("arbitrary",),
            vmem_limit_bytes=100 * 1024 * 1024,
        ),
        name="adaln_kernel",
    )(A_x.reshape(S, D), A_wqkv, A_wo, B_w1.T, B_b1, B_w2, B_b2, c, w_mod)
    return out.reshape(1, S, D)
```

```python
import functools
import math

import jax
import jax.numpy as jnp
from jax import lax
import jax.experimental.pallas as pl
import jax.experimental.pallas.tpu as pltpu

S = 2048
D = 640
H = 32
DH = 20
F = 1728
FM = 1664
TM = 256
NB = S // TM
QB = 128
NQ = TM // QB
NG = 8
NSLOT = 5
EPS = 1e-5
QSCALE = (DH ** -0.5) * math.log2(math.e)
NEG = -1e30
f32 = jnp.float32
bf16 = jnp.bfloat16
u32 = jnp.uint32
NT = (((1,), (1,)), ((), ()))
NN = (((1,), (0,)), ((), ()))


def _pk(a):
    return pltpu.bitcast(a.astype(bf16), u32)


def _upk(a):
    return pltpu.bitcast(a, bf16)


def _mm(a, b, dims=NN):
    return lax.dot_general(a, b, dims, preferred_element_type=f32)


def _ln(x):
    mu = jnp.mean(x, axis=-1, keepdims=True)
    xc = x - mu
    var = jnp.mean(xc * xc, axis=-1, keepdims=True)
    return xc * lax.rsqrt(var + EPS)


def _group_tiles(a):
    lane = lax.broadcasted_iota(jnp.int32, (a.shape[0], 128), 1)
    t = [a[:, 128 * j:128 * (j + 1)] for j in range(5)]
    out = []
    for g in range(NG):
        lo_t, hi_t = (80 * g) // 128, (80 * g + 79) // 128
        out.append(t[lo_t] if lo_t == hi_t else jnp.where(lane >= 64, t[lo_t], t[hi_t]))
    return out


def _kernel(x_hbm, wqkv_hbm, wo_hbm, w1T_hbm, b1_hbm, w2_hbm, b2_hbm, c_hbm, wmod_hbm,
            o_hbm,
            x_ref, wqkv_ref, wo_ref, w1T_ref, w2_ref, wmod_ref, b1_ref, b2_ref, c_ref,
            sc_ref, mod_ref, bias_ref, wT_ref, k_ref, q_ref, vT_ref, oT_ref, y_ref, x1_ref, o_ref, s_ref, kf_ref,
            sem):
    i = pl.program_id(0)

    def x_copy(b, s, n=1):
        return pltpu.make_async_copy(x_hbm.at[pl.ds(b * TM, n * TM)], x_ref.at[pl.ds(b * TM, n * TM)], sem.at[s])

    def o_copy(b, c0=0, c1=D):
        return pltpu.make_async_copy(o_ref.at[pl.ds(b * TM, TM), pl.ds(c0, c1 - c0)],
                                     o_hbm.at[pl.ds(b * TM, TM), pl.ds(c0, c1 - c0)], sem.at[2])

    def col_copy(src, dst, c0, n, s):
        return pltpu.make_async_copy(src.at[:, pl.ds(c0, n)], dst.at[:, pl.ds(c0, n)], sem.at[s])

    cp_first = (pltpu.make_async_copy(c_hbm, c_ref, sem.at[0]), x_copy(0, 0, 2))
    cp_ca = col_copy(wmod_hbm, wmod_ref, D, D, 1)
    cp_wk = col_copy(wqkv_hbm, wqkv_ref, D, D, 2)
    cp_q = (col_copy(wqkv_hbm, wqkv_ref, 0, D, 3), col_copy(wmod_hbm, wmod_ref, 0, D, 3))
    cp_wv = col_copy(wqkv_hbm, wqkv_ref, 2 * D, D, 4)
    cp_mid = (col_copy(wmod_hbm, wmod_ref, 2 * D, 4 * D, 5),
              pltpu.make_async_copy(wo_hbm, wo_ref, sem.at[5]),
              pltpu.make_async_copy(b1_hbm, b1_ref, sem.at[5]),
              pltpu.make_async_copy(b2_hbm, b2_ref, sem.at[5]))
    cp_late = (pltpu.make_async_copy(w1T_hbm, w1T_ref, sem.at[0]),
               pltpu.make_async_copy(w2_hbm, w2_ref, sem.at[0]),
               x_copy(2, 0))
    cp_xr = x_copy(3, 1, NB - 3)

    def modrow(k):
        return mod_ref[0:1, k * D:(k + 1) * D]

    def mod_span(c0, c1):
        mod_ref[:, c0:c1] = _mm(sc_ref[...], wmod_ref[:, c0:c1])

    def mod_cols(k0, k1):
        mod_span(k0 * D, k1 * D)

    def next_h(b, ch):
        hs = []
        for r0 in range(0, TM, ch):
            xc = x_ref[pl.ds(pl.multiple_of(b * TM + r0, ch), ch), :].astype(f32)
            hs.append(_ln(xc) * (1.0 + modrow(1)) + modrow(0))
        return jnp.concatenate(hs, axis=0)

    def store_q(qT, b):
        qTp = _pk(qT * QSCALE)
        r8 = lax.broadcasted_iota(jnp.int32, (8, QB), 0)
        for j in range(NQ):
            for g in range(NG):
                for v in range(5):
                    rows = slice(40 * g + 8 * v, 40 * g + 8 * v + 8)
                    blk = qTp[rows, QB * j:QB * (j + 1)]
                    k0, k1 = (8 * v) // 10, (8 * v + 7) // 10
                    rl = lambda k: blk if k == 0 else pltpu.roll(blk, 32 * k, 1)
                    val = rl(k0) if k0 == k1 else jnp.where(r8 + 8 * v < 10 * k1, rl(k0), rl(k1))
                    q_ref[b * NQ + j, rows, :] = val

    def store_v(vT, b):
        r24 = lax.broadcasted_iota(jnp.int32, (24, QB), 0)
        for hd in range(H):
            base = (20 * hd) // 8 * 8
            off = 20 * hd - base
            useful = (r24 >= off) & (r24 < off + 20)
            for j in range(NQ):
                win = vT[base:base + 24, QB * j:QB * (j + 1)]
                vT_ref[b * NQ + j, 24 * hd:24 * (hd + 1), :] = jnp.where(useful, win, 1.0)

    def store_k(k, b, r0=0):
        kt = _group_tiles(_pk(k))
        for g in range(NG):
            k_ref[(b * TM + r0) // 2:(b * TM + r0 + k.shape[0]) // 2, 128 * g:128 * (g + 1)] = kt[g]

    def proj_q(h, b):
        store_q(_mm(_upk(wT_ref[0:D // 2, :]), h, NT), b)

    def proj_v(h, b):
        store_v(_mm(_upk(wT_ref[D // 2:D, :]), h, NT), b)

    def attention(items, lag, keep=None, hook=None):
        r32 = lax.broadcasted_iota(jnp.int32, (32, 128), 0)
        l32 = lax.broadcasted_iota(jnp.int32, (32, 128), 1)
        tri = r32 > (l32 & 31)
        g_odd = (l32 & 32) != 0
        g_hi = l32 >= 64
        r16 = lax.broadcasted_iota(jnp.int32, (16, 128), 0)
        lg16 = lax.broadcasted_iota(jnp.int32, (16, 128), 1) >> 5
        kj = lax.broadcasted_iota(jnp.int32, (QB, QB), 0)
        qi = lax.broadcasted_iota(jnp.int32, (QB, QB), 1)
        uppers = [kj > ((qi - 32 * k) & 127) for k in range(4)]

        def stage_qk(n, jb, g):
            nk = min(jb + 1, 3)

            def krows(tile, a, cnt):
                st = (jb - 2 + tile) * 64 + a // 2
                return k_ref[st:st + cnt // 2, 128 * g:128 * (g + 1)]

            qx = _upk(q_ref[jb, 40 * g:40 * (g + 1), :]).astype(f32)

            def stat(heads, r):
                blocks = [None] * 8
                for v in range(5):
                    lo_r, hi_r = 16 * v, 16 * v + 16
                    msk = None
                    for k in heads:
                        if max(lo_r, 20 * k) >= min(hi_r, 20 * k + 20):
                            continue
                        rr = r16 + lo_r
                        mk = (rr >= 20 * k) & (rr < 20 * k + 20)
                        if r is not None:
                            mk = mk & (lg16 == (r + k) % 4)
                        msk = mk if msk is None else (msk | mk)
                    if msk is not None:
                        blocks[(5 * g + v) % 8] = jnp.where(msk, qx[lo_r:hi_r], 0.0)
                z = jnp.zeros((16, 128), f32)
                return jnp.concatenate([z if b_ is None else b_ for b_ in blocks], axis=0).astype(bf16)

            sq = [None] * 4
            for r in (range(4) if (nk == 3 or g % 2 == 0) else range(3, -1, -1)):
                parts, idx = [], []
                for c in range(4):
                    if c >= r and nk == 3:
                        parts.append(krows(0, 32 * c, 32))
                        idx.append((c, 0))
                    if c <= r:
                        parts.append(krows(2, 32 * c, 32))
                        idx.append((c, 2))
                s = _mm(_upk(jnp.concatenate(parts, axis=0)), stat(range(4), r))
                piece = {key: s[32 * m:32 * m + 32] for m, key in enumerate(idx)}
                neg = jnp.full((32, 128), NEG, f32)
                sq[r] = [piece[(c, 2)] if c < r else
                         (jnp.where(tri, piece.get((c, 0), neg), piece[(c, 2)]) if c == r else piece.get((c, 0), neg))
                         for c in range(4)]
            m8 = [None] * 4
            slot0 = (n % NSLOT) * 4
            for c in range(4):
                tt = [sq[(-k) % 4][c] for k in range(4)]
                uu = [jnp.where(g_odd, tt[(k - 1) % 4], tt[k]) for k in range(4)]
                for k in range(4):
                    sk = jnp.where(g_hi, uu[(k - 2) % 4], uu[k])
                    s_ref[slot0 + k, 32 * c:32 * c + 32] = sk
                    mc = jnp.maximum(jnp.maximum(sk[0:8], sk[8:16]), jnp.maximum(sk[16:24], sk[24:32]))
                    m8[k] = mc if m8[k] is None else jnp.maximum(m8[k], mc)
            yield None
            if nk >= 2:
                k1 = _upk(krows(1, 0, 128))
                s_mid = [_mm(k1, stat([k], None)) for k in range(4)]
            mx = []
            for k in range(4):
                if nk >= 2:
                    s1 = s_mid[k]
                    s_ref[slot0 + k, QB:2 * QB] = s1
                    for c in range(8):
                        m8[k] = jnp.maximum(m8[k], jnp.maximum(s1[16 * c:16 * c + 8], s1[16 * c + 8:16 * c + 16]))
                mx.append(jnp.max(m8[k], axis=0, keepdims=True))
            yield mx

        def stage_pv(n, jb, g, mx):
            nk = min(jb + 1, 3)
            slot0 = (n % NSLOT) * 4
            o = [None] * 4
            pm = [None] * 4

            def acc(k, tile, p):
                hd = 4 * g + k
                d = _mm(vT_ref[jb - 2 + tile, 24 * hd:24 * (hd + 1), :], p.astype(bf16))
                o[k] = d if o[k] is None else o[k] + d

            def merged(k):
                if pm[k] is None:
                    pm[k] = jnp.exp2(s_ref[slot0 + k, 0:QB] - mx[k])
                return pm[k]

            for tile in (2, 0, 1):
                for k in range(4):
                    if tile == 2:
                        acc(k, 2, jnp.where(uppers[k], 0.0, merged(k)) if nk == 3 else merged(k))
                    elif tile == 0 and nk == 3:
                        acc(k, 0, jnp.where(uppers[k], merged(k), 0.0))
                    elif tile == 1 and nk >= 2:
                        acc(k, 1, jnp.exp2(s_ref[slot0 + k, QB:2 * QB] - mx[k]))
                yield None
            for k in range(4):
                hd = 4 * g + k
                off = (20 * hd) % 8
                den = o[k][20:21] if off == 0 else o[k][0:1]
                r0 = pl.reciprocal(den, approx=True)
                on = o[k] * (r0 * (2.0 - den * r0))
                if k:
                    on = pltpu.roll(on, 128 - 32 * k, 1)
                oT_ref[20 * hd:20 * hd + 20, QB * jb:QB * (jb + 1)] = on[off:off + 20]

        def run_pv(args):
            for _ in stage_pv(*args):
                pass

        pend = []
        for n, it in enumerate(items):
            qk = stage_qk(n, *it)
            pv = stage_pv(*pend.pop(0)) if len(pend) >= lag else iter(())
            next(qk)
            next(pv, None)
            next(pv, None)
            pend.append((n, *it, next(qk)))
            for _ in pv:
                pass
            if keep is not None and len(pend) > keep + (len(items) - 1 - n) and len(pend) > 1:
                run_pv(pend.pop(0))
            if hook is not None:
                hook(n)
        return [functools.partial(run_pv, args) for args in pend]

    def block_items(blk, j_inner):
        if j_inner:
            return [(blk * NQ + j, g) for g in range(NG) for j in range(NQ)]
        return [(blk * NQ + j, g) for j in range(NQ) for g in range(NG)]

    def attn_rows(slot):
        return oT_ref[:, slot * TM:(slot + 1) * TM].T

    def post_attn(o_att, b, r0, r1, ch):
        attn = _mm(o_att[r0:r1].astype(bf16), wo_ref[...])
        xb = x_ref[pl.ds(pl.multiple_of(b * TM + r0, 16), r1 - r0), :].astype(f32)
        x1_ref[b % 2, r0:r1] = xb + modrow(2) * attn
        for c0 in range(r0, r1, ch):
            h2 = _ln(x1_ref[b % 2, c0:c0 + ch, :]) * (1.0 + modrow(4)) + modrow(3)
            y_ref[c0 // 2:(c0 + ch) // 2, :] = _pk(_ln(h2))

    def mlp_up(between=()):
        y = _upk(y_ref[...])
        parts, c0 = [], 0
        for fn in between:
            parts.append(_mm(y, w1T_ref[c0:c0 + 384, :], NT))
            c0 += 384
            fn()
        parts.append(_mm(y, w1T_ref[c0:FM, :], NT))
        parts.append(_mm(w1T_ref[FM:F, :], y, NT).T)
        a = jnp.concatenate(parts, axis=1)
        return jax.nn.gelu(a + bias_ref[0:1, 0:F], approximate=True).astype(bf16)

    def mlp_down(gl, b, c0, c1):
        mlp = _mm(gl, w2_ref[:, c0:c1])
        res = x1_ref[b % 2, :, c0:c1] + mod_ref[0:1, 5 * D + c0:5 * D + c1] * (mlp + bias_ref[1:2, c0:c1])
        o_ref[pl.ds(pl.multiple_of(b * TM, TM), TM), c0:c1] = res.astype(o_ref.dtype)

    @pl.when(i == 0)
    def _():
        for cp in (*cp_first, cp_ca, cp_wk, *cp_q, cp_wv, *cp_mid):
            cp.start()
        for cp in cp_first:
            cp.wait()
        for cp in cp_late:
            cp.start()
        cf = c_ref[...].astype(f32)
        sc_ref[...] = jnp.broadcast_to(cf * jax.nn.sigmoid(cf), (8, D))
        for b in range(2):
            x1_ref[b] = _ln(x_ref[b * TM:(b + 1) * TM, :].astype(f32))
        cp_ca.wait()
        cp_xr.start()
        mod_cols(1, 2)
        for b in range(2):
            x1_ref[b] = x1_ref[b] * (1.0 + modrow(1))

        cp_wk.wait()
        for b in range(2):
            for r0 in range(0, TM, 64):
                kf_ref[b, r0:r0 + 64] = _mm(x1_ref[b, r0:r0 + 64].astype(bf16), wqkv_ref[:, D:2 * D])
        for cp in cp_q:
            cp.wait()
        mod_cols(0, 1)
        wT_ref[0:D // 2, :] = _pk(wqkv_ref[:, 0:D].astype(f32).T)
        h = (x1_ref[0] + modrow(0)).astype(bf16)
        hn = (x1_ref[1] + modrow(0)).astype(bf16)
        q0T = jnp.concatenate([_mm(_upk(wT_ref[r0:r0 + D // 4, :]), h, NT) for r0 in (0, D // 4)], axis=0)
        kb = _mm(mod_ref[:, 0:D], wqkv_ref[:, D:2 * D])[0:1]
        cp_wv.wait()
        store_q(q0T, 0)
        wT_ref[D // 2:D, :] = _pk(wqkv_ref[:, 2 * D:3 * D].astype(f32).T)
        store_k(kf_ref[0] + kb, 0)
        store_k(kf_ref[1] + kb, 1)
        proj_q(hn, 1)
        proj_v(h, 0)
        proj_v(hn, 1)

        def wait_mid():
            for cp in cp_mid:
                cp.wait()
            bias_ref[0:1, 0:F] = b1_ref[...].astype(f32).reshape(1, F)
            bias_ref[1:2, 0:D] = b2_ref[...].astype(f32).reshape(1, D)

        def hook(n):
            if n == 13:
                wait_mid()
            if 13 <= n < 23:
                for m in (2 * (n - 13), 2 * (n - 13) + 1):
                    mod_span(2 * D + 128 * m, 2 * D + 128 * (m + 1))
            if 21 <= n < 25:
                post_attn(attn_rows(0), 0, 64 * (n - 21), 64 * (n - 20), 32)

        for t in attention(block_items(0, True) + block_items(1, True), 3, 1, hook):
            t()
        for cp in cp_late:
            cp.wait()

    @pl.when(i == 2)
    def _():
        cp_xr.wait()

    @pl.when(jnp.logical_and(i > 0, i < NB - 1))
    def _():
        k_ref[0:TM // 2, :] = k_ref[TM // 2:TM, :]
        vT_ref[0:NQ] = vT_ref[NQ:2 * NQ]
        hf = next_h(i + 1, 32)
        hn = hf.astype(bf16)

        def k_rows(r0):
            store_k(_mm(hf[r0:r0 + 64].astype(bf16), wqkv_ref[:, D:2 * D]), 1, r0)
            if r0 == TM - 64:
                proj_q(hn, 1)

        gl = mlp_up([functools.partial(k_rows, r0) for r0 in range(0, TM, 64)])
        o_att = attn_rows(1)
        for n in range(3):
            post_attn(o_att, i, 64 * n, 64 * (n + 1), 64)
        v_lo = _mm(_upk(wT_ref[D // 2:3 * D // 4, :]), hn, NT)
        post_attn(o_att, i, 192, TM, 64)
        v_hi = _mm(_upk(wT_ref[3 * D // 4:D, :]), hn, NT)
        store_v(jnp.concatenate([v_lo, v_hi], axis=0), 1)
        tail = attention(block_items(1, False), 2)
        for n in range(5):
            if n < len(tail):
                tail[n]()
            mlp_down(gl, i - 1, 128 * n, 128 * (n + 1))
        o_copy(i - 1).start()

    @pl.when(i == NB - 1)
    def _():
        gl = mlp_up()
        o_att = attn_rows(1)
        for n in range(5):
            if n < 4:
                post_attn(o_att, NB - 1, 64 * n, 64 * (n + 1), 64)
            mlp_down(gl, NB - 2, 128 * n, 128 * (n + 1))
        o_copy(NB - 2).start()
        gl = mlp_up()
        chunks = ((0, 256), (256, 512), (512, D))
        for c0, c1 in chunks:
            mlp_down(gl, NB - 1, c0, c1)
            o_copy(NB - 1, c0, c1).start()
        for b in range(NB - 1):
            o_copy(b).wait()
        for c0, c1 in chunks:
            o_copy(NB - 1, c0, c1).wait()


@jax.jit
def pallas_adaLN_cond__sliding_block__mixer_channel_mlp__prompt_kernel(
    A_x: jax.Array,
    A_wqkv: jax.Array,
    A_wo: jax.Array,
    B_x: jax.Array,
    B_w1: jax.Array,
    B_b1: jax.Array,
    B_w2: jax.Array,
    B_b2: jax.Array,
    c: jax.Array,
    w_mod: jax.Array,
):
    del B_x
    hbm = pl.BlockSpec(memory_space=pl.ANY)
    out = pl.pallas_call(
        _kernel,
        grid=(NB,),
        in_specs=[hbm] * 9,
        out_specs=hbm,
        out_shape=jax.ShapeDtypeStruct((S, D), A_x.dtype),
        scratch_shapes=[
            pltpu.VMEM((S, D), bf16),
            pltpu.VMEM((D, 3 * D), bf16),
            pltpu.VMEM((D, D), bf16),
            pltpu.VMEM((F, D), bf16),
            pltpu.VMEM((F, D), bf16),
            pltpu.VMEM((D, 6 * D), bf16),
            pltpu.VMEM((F,), bf16),
            pltpu.VMEM((D,), bf16),
            pltpu.VMEM((1, D), bf16),
            pltpu.VMEM((8, D), f32),
            pltpu.VMEM((8, 6 * D), f32),
            pltpu.VMEM((8, F), f32),
            pltpu.VMEM((D, D), u32),
            pltpu.VMEM((TM, NG * 128), u32),
            pltpu.VMEM((2 * NQ, D // 2, QB), u32),
            pltpu.VMEM((2 * NQ, H * 24, QB), f32),
            pltpu.VMEM((D, 2 * TM), f32),
            pltpu.VMEM((TM // 2, D), u32),
            pltpu.VMEM((2, TM, D), f32),
            pltpu.VMEM((S, D), bf16),
            pltpu.VMEM((NSLOT * 4, 2 * QB, QB), f32),
            pltpu.VMEM((2, TM, D), f32),
            pltpu.SemaphoreType.DMA((6,)),
        ],
        compiler_params=pltpu.CompilerParams(
            dimension_semantics=("arbitrary",),
            vmem_limit_bytes=100 * 1024 * 1024,
        ),
        name="adaln_kernel",
    )(A_x.reshape(S, D), A_wqkv, A_wo, B_w1.T, B_b1, B_w2, B_b2, c, w_mod)
    return out.reshape(1, S, D)
```
